```python
import jax
import jax.numpy as jnp

def _softmax(x, axis=-1):
    return jax.nn.softmax(x, axis=axis)

def _gelu(x):
    return jax.nn.gelu(x, approximate=True)

def _silu(x):
    return jax.nn.silu(x)

def _sigmoid(x):
    return jax.nn.sigmoid(x)

def _layernorm(x, axis=-1, eps=1e-05):
    m = jnp.mean(x, axis=axis, keepdims=True)
    v = jnp.var(x, axis=axis, keepdims=True)
    return (x - m) / jnp.sqrt(v + eps)

def _scatter_add(tgt, idx, src, axis=0):
    return tgt.at[idx].add(src)

def _segment_sum(src, seg, n):
    return jax.ops.segment_sum(src, seg, n)

class _Rng:

    def __init__(self, key):
        self._k = key

    def _next(self):
        self._k, sub = jax.random.split(self._k)
        return sub

    def normal(self, shape):
        return jax.random.normal(self._next(), shape, dtype=jnp.bfloat16)

    def randint(self, lo, hi, shape):
        return jax.random.randint(self._next(), shape, lo, hi, dtype=jnp.int32)

    def uniform(self, shape, lo=0.0, hi=1.0):
        return jax.random.uniform(self._next(), shape, jnp.bfloat16, lo, hi)

    def permutation(self, n):
        return jax.random.permutation(self._next(), n)
kernel_name = 'interleave_layers__memory_aug_infini_attn__sliding_local_dilated__prompt'

def setup_inputs():
    _rng = _Rng(jax.random.key(int.from_bytes(__import__("os").urandom(4), "little")))
    _w = lambda a: (lambda t: t.astype(jnp.bfloat16) if jnp.issubdtype(t.dtype, jnp.floating) else t)(jnp.asarray(a))

    def _A_setup():
        B, S, D, H = (1, 2048, 1024, 32)
        N = 4
        L = max(1, S // N)
        sc = D ** (-0.5)
        return {'x': _w((lambda *s: _rng.normal(s) * 0.05)(B, N * L, D)), 'wq': _w((lambda *s: _rng.normal(s) * 0.05)(D, D) * sc), 'wk': _w((lambda *s: _rng.normal(s) * 0.05)(D, D) * sc), 'wv': _w((lambda *s: _rng.normal(s) * 0.05)(D, D) * sc), 'wo': _w((lambda *s: _rng.normal(s) * 0.05)(D, D) * sc), 'beta': _w((lambda *s: _rng.normal(s) * 0.05)(H))}
    _A_in = _A_setup()

    def _B_setup():
        B, S, D = (1, 2048, 1024)
        return {'x': _w((lambda *s: _rng.normal(s) * 0.05)(B, S, D)), 'wqkv': _w((lambda *s: _rng.normal(s) * 0.05)(D, 3 * D)), 'wo': _w((lambda *s: _rng.normal(s) * 0.05)(D, D))}
    _B_in = _B_setup()
    return {'A_x': _A_in['x'], 'A_wq': _A_in['wq'], 'A_wk': _A_in['wk'], 'A_wv': _A_in['wv'], 'A_wo': _A_in['wo'], 'A_beta': _A_in['beta'], 'B_x': _B_in['x'], 'B_wqkv': _B_in['wqkv'], 'B_wo': _B_in['wo']}

def reference(A_x, A_wq, A_wk, A_wv, A_wo, A_beta, B_x, B_wqkv, B_wo):

    def _A_ref(x, wq, wk, wv, wo, beta):
        B, S, D = x.shape
        H = 32
        Dh = D // H
        N = 4
        L = S // N
        q = (lambda x, *d: x.transpose(*d))((x @ wq).reshape(B, S, H, Dh), 0, 2, 1, 3).reshape(B, H, N, L, Dh)
        k = (lambda x, *d: x.transpose(*d))((x @ wk).reshape(B, S, H, Dh), 0, 2, 1, 3).reshape(B, H, N, L, Dh)
        v = (lambda x, *d: x.transpose(*d))((x @ wv).reshape(B, S, H, Dh), 0, 2, 1, 3).reshape(B, H, N, L, Dh)
        phi = lambda t: jnp.where(t > 0, t + 1.0, jnp.exp(t))
        scale = Dh ** (-0.5)
        ar = jnp.arange(L)
        mask = (lambda x, dt: x.astype(dt))(ar[:, None] < ar[None, :], x.dtype) * -1000000000.0
        g = _sigmoid(beta).reshape(1, H, 1, 1)
        M = jnp.einsum('bhd,bhe->bhde', q[:, :, 0, 0, :] * 0.0, q[:, :, 0, 0, :] * 0.0)
        z = q[:, :, 0, 0, :] * 0.0
        outs = []
        for s in range(N):
            qs, ks, vs = (q[:, :, s].copy(), k[:, :, s].copy(), v[:, :, s].copy())
            logits = jnp.einsum('bhqd,bhkd->bhqk', qs, ks) * scale + mask
            p = _softmax(logits, axis=-1)
            a_dot = jnp.einsum('bhqk,bhkd->bhqd', p, vs)
            pq = phi(qs)
            num = jnp.einsum('bhld,bhde->bhle', pq, M)
            den = jnp.einsum('bhld,bhd->bhl', pq, z)[..., None] + 1e-06
            a_mem = num / den
            o = g * a_mem + (1.0 - g) * a_dot
            outs.append(o)
            pk = phi(ks)
            M = M + jnp.einsum('bhld,bhle->bhde', pk, vs)
            z = z + jnp.einsum('bhld->bhd', pk)
        o = (lambda x, *d: x.transpose(*d))(jnp.stack(outs, 2).reshape(B, H, S, Dh), 0, 2, 1, 3).reshape(B, S, D)
        return o @ wo

    def _B_ref(x, wqkv, wo):
        B, S, D = x.shape
        H = 32
        Dh = D // H
        W, dil = (8, 2)
        qkv = (lambda x, *d: x.transpose(*d))((x @ wqkv).reshape(B, S, 3, H, Dh), 2, 0, 3, 1, 4)
        q, k, v = (qkv[0], qkv[1], qkv[2])
        scale = Dh ** (-0.5)
        pos = jnp.arange(S)
        off = jnp.arange(W) * dil
        idx = pos[:, None] - off[None, :]
        mask = idx >= 0
        idx_c = jnp.where(mask, idx, 0).reshape(-1)
        kg = k[:, :, idx_c, :].reshape(B, H, S, W, Dh)
        vg = v[:, :, idx_c, :].reshape(B, H, S, W, Dh)
        logits = jnp.einsum('bhsd,bhswd->bhsw', q, kg) * scale
        logits = jnp.where(mask[None, None, :, :], logits, -1000000000.0)
        attn = _softmax(logits, axis=-1)
        o = jnp.einsum('bhsw,bhswd->bhsd', attn, vg)
        return (lambda x, *d: x.transpose(*d))(o, 0, 2, 1, 3).reshape(B, S, D) @ wo
    x = A_x
    x = x + _A_ref(_layernorm(x, axis=-1), A_wq, A_wk, A_wv, A_wo, A_beta)
    x = x + _B_ref(_layernorm(x, axis=-1), B_wqkv, B_wo)
    x = x + _A_ref(_layernorm(x, axis=-1), A_wq, A_wk, A_wv, A_wo, A_beta)
    x = x + _B_ref(_layernorm(x, axis=-1), B_wqkv, B_wo)
    return x
```

```python
import functools
import math

import jax
import jax.numpy as jnp
import numpy as np
from jax import lax
from jax.experimental import pallas as pl
from jax.experimental.pallas import tpu as pltpu

S, D, H, DH = 2048, 1024, 32, 32
L = 512
NSEG = S // L
NG = D // 128
W, DIL = 8, 2
HALO = 16
LOG2E = math.log2(math.e)
F32, BF16 = jnp.float32, jnp.bfloat16
NN = (((1,), (0,)), ((), ()))
NT = (((1,), (1,)), ((), ()))


def _mm(a, b, dims=NN):
    return lax.dot_general(a, b, dims, preferred_element_type=F32)


def _layernorm(x):
    m = jnp.mean(x, axis=-1, keepdims=True)
    xc = x - m
    v = jnp.mean(xc * xc, axis=-1, keepdims=True)
    return xc * lax.rsqrt(v + 1e-5)


def _phi(t):
    return jnp.where(t > 0, t + 1.0, jnp.exp(t))


def _kernel(x_ref, beta_ref, awq_h, awk_h, awv_h, awo_h, bwqkv_h, bwo_h, out_ref,
            wq_s, wk_s, wv_raw, wvt_s, awo_s, bw_raw, bwt_s, bwo_raw, bwo_s, tmp_s,
            gate_s, x_s, ln_s, o_s, mt_s, z_s, q_b, k_b, v_b, kt_s, vt_s, sems):
    seg = pl.program_id(0)
    rep = pl.program_id(1)
    first = jnp.logical_and(seg == 0, rep == 0)

    def weight_copies():
        cps = [pltpu.make_async_copy(awv_h, wv_raw, sems.at[0]),
               pltpu.make_async_copy(awq_h, wq_s, sems.at[1]),
               pltpu.make_async_copy(awk_h, wk_s, sems.at[2]),
               pltpu.make_async_copy(awo_h, awo_s, sems.at[3]),
               pltpu.make_async_copy(bwqkv_h, bw_raw, sems.at[4]),
               pltpu.make_async_copy(bwo_h, bwo_raw, sems.at[5])]
        return cps

    @pl.when(first)
    def _():
        cps = weight_copies()
        for c in cps:
            c.start()
        g = jax.nn.sigmoid(beta_ref[...].astype(F32).reshape(1, H))
        r = lax.broadcasted_iota(jnp.int32, (H, H), 0)
        c_ = lax.broadcasted_iota(jnp.int32, (H, H), 1)
        gcol = jnp.sum(jnp.where(r == c_, jnp.broadcast_to(g, (H, H)), 0.0), axis=1, keepdims=True)
        gate_s[...] = jnp.broadcast_to(gcol, (H, 128))
        cps[0].wait()

        def tr(i, _):
            c0 = pl.multiple_of(i * 128, 128)
            wvt_s[pl.ds(c0, 128), :] = wv_raw[:, pl.ds(c0, 128)].T
        lax.fori_loop(0, NG, tr, None)
        cps[1].wait()
        cps[2].wait()
        cps[3].wait()

    @pl.when(seg == 0)
    def _():
        mt_s[rep] = jnp.zeros(mt_s.shape[1:], F32)
        z_s[rep] = jnp.zeros(z_s.shape[1:], F32)
        kt_s[rep] = jnp.zeros(kt_s.shape[1:], F32)
        vt_s[rep] = jnp.zeros(vt_s.shape[1:], F32)

    @pl.when(rep == 0)
    def _():
        x = x_ref[...].astype(F32)
        x_s[...] = x
        ln_s[...] = _layernorm(x).astype(BF16)

    lane = lax.broadcasted_iota(jnp.int32, (128, 128), 1)
    row = lax.broadcasted_iota(jnp.int32, (128, 128), 0)
    same_head = (lane // DH) == (row // DH)
    causal = row <= lane
    lane16 = lax.broadcasted_iota(jnp.int32, (16, 128), 1)
    row16 = lax.broadcasted_iota(jnp.int32, (16, 128), 0)

    def a_group(g, _):
        c0 = pl.multiple_of(g * 128, 128)
        ln = ln_s[...]
        q = _mm(ln, wq_s[:, pl.ds(c0, 128)])
        k = _mm(ln, wk_s[:, pl.ds(c0, 128)])
        vt = _mm(wvt_s[pl.ds(c0, 128), :], ln, NT).astype(BF16)
        qs = q * (DH ** -0.5 * LOG2E)
        kb = k.astype(BF16)
        pq = _phi(q).astype(BF16)
        pk = _phi(k)
        mt = mt_s[rep, g]
        z = z_s[rep, g]
        zs = jnp.sum(z, axis=0, keepdims=True)
        zrows = jnp.where(lane16 // DH == row16, jnp.broadcast_to(zs, (16, 128)), 0.0)
        maug = jnp.concatenate([mt, zrows], axis=0).astype(BF16)
        numt = _mm(maug, pq, NT)
        mt_s[rep, g] = mt + jnp.where(same_head, _mm(vt, pk.astype(BF16)), 0.0)
        z_s[rep, g] = z + jnp.sum(pk.reshape(L // 8, 8, 128), axis=0)
        for j in range(L // 128):
            qj = qs[j * 128:(j + 1) * 128]
            nk = (j + 1) * 128
            outs = []
            for h in range(4):
                qm = jnp.where(lane // DH == h, qj, 0.0).astype(BF16)
                st = _mm(kb[:nk], qm, NT)
                sd = jnp.where(causal, st[nk - 128:], -1e30)
                st = sd if j == 0 else jnp.concatenate([st[:nk - 128], sd], axis=0)
                m = jnp.max(st, axis=0, keepdims=True)
                p = jnp.exp2(st - m)
                l = jnp.sum(p, axis=0, keepdims=True)
                ot = _mm(vt[h * DH:(h + 1) * DH, :nk], p.astype(BF16))
                gate = gate_s[pl.ds(g * 4 + h, 1), :]
                den = numt[128 + h:128 + h + 1, j * 128:(j + 1) * 128] + 1e-6
                num = numt[h * DH:(h + 1) * DH, j * 128:(j + 1) * 128]
                outs.append(ot * ((1.0 - gate) / l) + num * (gate / den))
            o_s[j * 128:(j + 1) * 128, pl.ds(c0, 128)] = jnp.concatenate(outs, axis=0).T.astype(BF16)

    lax.fori_loop(0, NG, a_group, None)

    x = x_s[...] + _mm(o_s[...], awo_s[...])
    x_s[...] = x
    ln_s[...] = _layernorm(x).astype(BF16)

    @pl.when(first)
    def _():
        cps = weight_copies()
        cps[4].wait()

        def perm_w(i, _):
            t = i // NG
            c0 = pl.multiple_of((i % NG) * 128, 128)
            n0 = pl.multiple_of(t * D, D)
            tmp_s[...] = bw_raw[pl.ds(c0, 128), pl.ds(n0, D)].astype(F32).T
            for d in range(DH):
                bwt_s[pl.ds(n0 + d * H, H), pl.ds(c0, 128)] = tmp_s[pl.ds(d, H, stride=DH), :].astype(BF16)
        lax.fori_loop(0, 3 * NG, perm_w, None)
        cps[5].wait()

        def perm_o(i, _):
            c0 = pl.multiple_of(i * 128, 128)
            tmp_s[...] = bwo_raw[:, pl.ds(c0, 128)].astype(F32)
            for d in range(DH):
                bwo_s[pl.ds(d * H, H), pl.ds(c0, 128)] = tmp_s[pl.ds(d, H, stride=DH), :].astype(BF16)
        lax.fori_loop(0, NG, perm_o, None)

    def b_proj(g, _):
        c0 = pl.multiple_of(g * 128, 128)
        ln = ln_s[...]
        q_b[g] = _mm(ln, bwt_s[pl.ds(c0, 128), :], NT) * (DH ** -0.5 * LOG2E)
        k = _mm(ln, bwt_s[pl.ds(D + c0, 128), :], NT)
        k_b[g, :HALO] = kt_s[rep, g]
        k_b[g, HALO:] = k
        kt_s[rep, g] = k[L - HALO:]
        v = _mm(ln, bwt_s[pl.ds(2 * D + c0, 128), :], NT)
        v_b[g, :HALO] = vt_s[rep, g]
        v_b[g, HALO:] = v
        vt_s[rep, g] = v[L - HALO:]
    lax.fori_loop(0, NG, b_proj, None)

    RB = 16

    def b_attn(i, _):
        r0 = pl.multiple_of(i * RB, RB)
        pos = seg * L + r0 + lax.broadcasted_iota(jnp.int32, (RB, 128), 0)
        lg = []
        for w in range(W):
            acc = None
            for g in range(NG):
                t = q_b[g, pl.ds(r0, RB), :] * k_b[g, pl.ds(r0 + HALO - DIL * w, RB), :]
                acc = t if acc is None else acc + t
            acc = acc + pltpu.roll(acc, 64, 1)
            acc = acc + pltpu.roll(acc, 32, 1)
            if w:
                acc = jnp.where(pos >= DIL * w, acc, -1e9 * LOG2E)
            lg.append(acc)
        m = functools.reduce(jnp.maximum, lg)
        p = [jnp.exp2(t - m) for t in lg]
        inv = 1.0 / functools.reduce(jnp.add, p)
        p = [t * inv for t in p]
        for g in range(NG):
            acc = None
            for w in range(W):
                t = p[w] * v_b[g, pl.ds(r0 + HALO - DIL * w, RB), :]
                acc = t if acc is None else acc + t
            o_s[pl.ds(r0, RB), g * 128:(g + 1) * 128] = acc.astype(BF16)
    lax.fori_loop(0, L // RB, b_attn, None)

    x = x_s[...] + _mm(o_s[...], bwo_s[...])
    x_s[...] = x
    ln_s[...] = _layernorm(x).astype(BF16)
    out_ref[...] = x.astype(out_ref.dtype)


@jax.jit
def pallas_interleave_layers__memory_aug_infini_attn__sliding_local_dilated__prompt_kernel(
        A_x, A_wq, A_wk, A_wv, A_wo, A_beta, B_x, B_wqkv, B_wo):
    del B_x
    hbm = pl.BlockSpec(memory_space=pl.ANY)
    scratch = [
        pltpu.VMEM((D, D), BF16), pltpu.VMEM((D, D), BF16), pltpu.VMEM((D, D), BF16), pltpu.VMEM((D, D), BF16),
        pltpu.VMEM((D, D), BF16),
        pltpu.VMEM((D, 3 * D), BF16), pltpu.VMEM((3 * D, D), BF16),
        pltpu.VMEM((D, D), BF16), pltpu.VMEM((D, D), BF16),
        pltpu.VMEM((D, 128), F32),
        pltpu.VMEM((H, 128), F32),
        pltpu.VMEM((L, D), F32), pltpu.VMEM((L, D), BF16), pltpu.VMEM((L, D), BF16),
        pltpu.VMEM((2, NG, 128, 128), F32), pltpu.VMEM((2, NG, 8, 128), F32),
        pltpu.VMEM((NG, L, 128), F32), pltpu.VMEM((NG, L + HALO, 128), F32), pltpu.VMEM((NG, L + HALO, 128), F32),
        pltpu.VMEM((2, NG, HALO, 128), F32), pltpu.VMEM((2, NG, HALO, 128), F32),
        pltpu.SemaphoreType.DMA((6,)),
    ]
    return pl.pallas_call(
        _kernel,
        grid=(NSEG, 2),
        in_specs=[pl.BlockSpec((None, L, D), lambda s, r: (0, s, 0)),
                  pl.BlockSpec((H,), lambda s, r: (0,)),
                  hbm, hbm, hbm, hbm, hbm, hbm],
        out_specs=pl.BlockSpec((None, L, D), lambda s, r: (0, s, 0)),
        out_shape=jax.ShapeDtypeStruct(A_x.shape, A_x.dtype),
        scratch_shapes=scratch,
        compiler_params=pltpu.CompilerParams(
            dimension_semantics=("arbitrary", "arbitrary"),
            vmem_limit_bytes=100 * 2 ** 20),
        name="interleaved_attn",
    )(A_x, A_beta, A_wq, A_wk, A_wv, A_wo, B_wqkv, B_wo)
```

```python
import functools
import math
import os

import jax
import jax.numpy as jnp
import numpy as np
from jax import lax
from jax.experimental import pallas as pl
from jax.experimental.pallas import tpu as pltpu

S, D, H, DH = 2048, 1024, 32, 32
L = 512
NSEG = S // L
NG = D // 128
NP = NG // 2
C = 128
NC = L // C
KH = D // 2
W, DIL = 8, 2
HALO = 16
LOG2E = math.log2(math.e)
QSCALE = DH ** -0.5 * LOG2E
F32, BF16, U32 = jnp.float32, jnp.bfloat16, jnp.uint32
NN = (((1,), (0,)), ((), ()))
NT = (((1,), (1,)), ((), ()))
cfg = lambda k, d: int(os.environ.get("KCFG_" + k, d))
LOOK = cfg("LOOK", 1)
RB = cfg("RB", 8)
P = functools.partial


def _mm(a, b, dims=NN):
    return lax.dot_general(a, b, dims, preferred_element_type=F32)


def _pack(x):
    if x.shape[1] == 128:
        n = x.shape[0] // 2
        y = _pack(jnp.concatenate([x[:n], x[n:]], axis=1))
        return jnp.concatenate([y[:, :128], y[:, 128:]], axis=0)
    return pltpu.bitcast(x.astype(BF16), U32)


def _pack_all(vs):
    y = _pack(jnp.concatenate(list(vs) + list(vs[:len(vs) % 2]), axis=1))
    return [y[:, i * 128:(i + 1) * 128] for i in range(len(vs))]


def _bf(x):
    return pltpu.bitcast(x, BF16)


def _layernorm(x):
    m = jnp.mean(x, axis=-1, keepdims=True)
    xc = x - m
    v = jnp.mean(xc * xc, axis=-1, keepdims=True)
    return xc * lax.rsqrt(v + 1e-5)


def _phi(t):
    return jnp.where(t > 0, t + 1.0, jnp.exp(t))


def _x_terms(x11, x12, x21, x22):
    return (x11 + x22, x21 + x22, x11, x22, x11 + x12, x21 - x11, x12 - x22)


def _w_terms(w11, w12, w21, w22):
    return (w11 + w22, w11, w12 - w22, w21 - w11, w22, w11 + w12, w21 + w22)


def _strassen_steps(prod, emit):
    m = {}

    def step(i):
        y = prod(i)
        if i == 1:
            m[1] = y
        elif i == 3:
            m[3] = y
            emit(1, 0, m[1] + y)
        elif i == 4:
            m[4] = y
            m["a"] = m.pop(3) - y
        elif i == 2:
            emit(0, 1, y + m.pop(4))
            m["b"] = y - m.pop(1)
        elif i == 0:
            m["a"] += y
            m["b"] += y
        elif i == 6:
            emit(0, 0, m.pop("a") + y)
        else:
            emit(1, 1, m.pop("b") + y)
        return y
    return [P(step, i) for i in (1, 3, 4, 2, 0, 6, 5)]


_CNT = [0]


def _weave(mxu, *side):
    after = [[] for _ in mxu]
    for steps in side:
        for i, f in enumerate(steps):
            pos = (i + 0.5) / len(steps) * len(mxu)
            after[int(pos)].append((pos % 1.0, f))

    def run():
        for f, todo in zip(mxu, after):
            y = f()
            for frac, g in sorted(todo, key=lambda t: t[0]):
                r = int(frac * (y.shape[0] // 8)) * 8
                g(y[r:r + 8, :128])
    if os.environ.get("KCFG_SCOPES"):
        _CNT[0] += 1
        with jax.named_scope("ph%02d" % _CNT[0]):
            run()
    else:
        run()


def _tile(g, n=1):
    if isinstance(g, int):
        return pl.ds(g * 128, n * 128)
    return pl.ds(pl.multiple_of(g * 128, 128), n * 128)


def _kernel(x_h, beta_ref, awq_h, awk_h, awv_h, awo_h, bwqkv_h, bwo_h, out_h,
            io_s, raw_a, raw_b, raw_o, tmp_s, wa_qk, wa_v, wb, wo,
            gate_s, x_s, x_new, xs, os_, mt_s, z_s, qs_a, pq_a, k_a, pk_a, vt_a,
            q_b, k_b, v_b, lg_b, p_b, o_cur, sems, *sc):
    def wcopy(i):
        src, dst = ((x_h.at[0], io_s), (awq_h, raw_a.at[0]), (awk_h, raw_a.at[1]), (awv_h, raw_a.at[2]),
                    (awo_h, raw_o.at[0]), (bwqkv_h, raw_b), (bwo_h, raw_o.at[1]))[i]
        return pltpu.make_async_copy(src, dst, sems.at[i])

    def out_copy(s):
        r = pl.ds(pl.multiple_of(s * L, L), L)
        return pltpu.make_async_copy(io_s.at[r], out_h.at[0, r], sems.at[7 + s])

    def ln_steps(s, r0, n, store, zero):
        def f(i, y):
            if y is not None:
                x_s[NSEG + zero, :8, :128] = y
            r = r0 + i * 16
            a = (r // C) * (2 * C) + r % C
            if not isinstance(r, int):
                a = pl.multiple_of(a, 16)
            y1 = _layernorm(x_s[s, pl.ds(a, 16)])
            y2 = _layernorm(x_s[s, pl.ds(a + C, 16)])
            for t, v in enumerate(_x_terms(y1[:, :KH], y1[:, KH:], y2[:, :KH], y2[:, KH:])):
                store(t, i, _pack(v))
        return [P(f, i) for i in range(n // 16)]

    for i in range(7):
        wcopy(i).start()
    g_ = jax.nn.sigmoid(beta_ref[...].astype(F32).reshape(1, H))
    r_ = lax.broadcasted_iota(jnp.int32, (H, H), 0)
    c_ = lax.broadcasted_iota(jnp.int32, (H, H), 1)
    gcol = jnp.sum(jnp.where(r_ == c_, jnp.broadcast_to(g_, (H, H)), 0.0), axis=1, keepdims=True)
    gate_s[...] = jnp.broadcast_to(gcol, (H, 128))
    os_[1] = jnp.zeros(os_.shape[1:], U32)
    wcopy(0).wait()

    def cvt(i, _):
        x_s[i // NC, pl.ds(pl.multiple_of(i % NC * C, C), C)] = io_s[pl.ds(pl.multiple_of(i * C, C), C)].astype(F32)
    lax.fori_loop(0, S // C, cvt, None)

    def ln0(i, _):
        def store(t, j, v):
            xs[0, t, pl.ds(pl.multiple_of(i * 32 + j * 8, 8), 8)] = v
        for f in ln_steps(0, i * 64, 64, store, 0):
            f(None)
    lax.fori_loop(0, 4, ln0, None)

    def u32(x):
        return lax.bitcast_convert_type(x.astype(F32), U32)

    def halves_t(w, k0, cols):
        return ((u32(w[pl.ds(k0, 128), cols]) >> 16) | u32(w[pl.ds(KH + k0, 128), cols])).T

    def split(p):
        return (lax.bitcast_convert_type(p << 16, F32),
                lax.bitcast_convert_type(p & np.uint32(0xFFFF0000), F32))

    wcopy(1).wait()
    wcopy(2).wait()

    def prep_qk(i, _):
        g, k0 = i // 4, pl.multiple_of(i % 4 * 128, 128)
        w = [raw_a[g % 2, pl.ds(k * KH + k0, 128), _tile(g // 2 * 2 + n)].astype(F32) for k in range(2) for n in range(2)]
        for t, v in enumerate(_w_terms(*w)):
            wa_qk[g, t, pl.ds(pl.multiple_of(k0 // 2, 64), 64)] = _pack(v)
    lax.fori_loop(0, 4 * NG, prep_qk, None)
    wcopy(3).wait()

    def prep_v(i, _):
        p, k0 = i // 4, pl.multiple_of(i % 4 * 128, 128)
        lo, hi = split(halves_t(raw_a.at[2], k0, _tile(2 * p, 2)))
        for t, v in enumerate(_w_terms(lo[:128], lo[128:], hi[:128], hi[128:])):
            wa_v[p, t, :, pl.ds(k0, 128)] = _pack(v)
    lax.fori_loop(0, 4 * NP, prep_v, None)
    wcopy(4).wait()

    def prep_o(i, _):
        p, kp = i // 4, i % 4
        w = [raw_o[0, _tile(2 * kp + k), _tile(2 * p + n)].astype(F32) for k in range(2) for n in range(2)]
        for t, v in enumerate(_w_terms(*w)):
            wo[0, p, t, pl.ds(pl.multiple_of(kp * 64, 64), 64)] = _pack(v)
    lax.fori_loop(0, 4 * NP, prep_o, None)
    wcopy(5).wait()

    def spread(i, v):
        for h in range(H):
            tmp_s[i, pl.ds(h * (DH + 1), DH)] = v[h * DH:(h + 1) * DH]

    def gather(i, g):
        return jnp.concatenate([tmp_s[i, pl.ds(4 * g + d, H, stride=DH + 1)] for d in range(4)], axis=0)

    def prep_b(i, _):
        k0 = pl.multiple_of(i * 128, 128)
        for t in range(3):
            spread(t, halves_t(raw_b, k0, pl.ds(t * D, D)))
        for j in range(NG + NP):
            n1, n2 = gather(j // NP, 2 * (j % NP)), gather(j // NP, 2 * (j % NP) + 1)
            (w11, w21), (w12, w22) = split(n1), split(n2)
            for t, v in enumerate(_w_terms(w11, w12, w21, w22)):
                wb[j, t, :, pl.ds(k0, 128)] = _pack(v)
    lax.fori_loop(0, 4, prep_b, None)
    wcopy(6).wait()

    def prep_bo(p, _):
        spread(0, (u32(raw_o[1, :, _tile(2 * p)]) >> 16) | u32(raw_o[1, :, _tile(2 * p + 1)]))
        for kp in range(NP):
            (w11, w12), (w21, w22) = split(gather(0, 2 * kp)), split(gather(0, 2 * kp + 1))
            for t, v in enumerate(_w_terms(w11, w12, w21, w22)):
                wo[1, p, t, pl.ds(kp * 64, 64)] = _pack(v)
    lax.fori_loop(0, NP, prep_bo, None)

    lane = lax.broadcasted_iota(jnp.int32, (128, 128), 1)
    row = lax.broadcasted_iota(jnp.int32, (128, 128), 0)
    same_head = (lane // DH) == (row // DH)
    causal = row <= lane
    lane64 = lax.broadcasted_iota(jnp.int32, (64, 128), 1)
    lane16 = lax.broadcasted_iota(jnp.int32, (16, 128), 1)
    row16 = lax.broadcasted_iota(jnp.int32, (16, 128), 0)

    def rows(c):
        return pl.ds(c * C, C)

    def prows(c):
        return pl.ds(c * C // 2, C // 2)

    def out_steps(s, layer, o_terms, p, final=False):
        def emit(rh, nh, y):
            for i in range(2):
                c = 2 * i + rh
                x = x_s[s, rows(c), _tile(2 * p + nh)] + y[i * C:(i + 1) * C]
                x_s[s, rows(c), _tile(2 * p + nh)] = x
                if final:
                    io_s[pl.ds(pl.multiple_of(s * L + c * C, C), C), _tile(2 * p + nh)] = x.astype(io_s.dtype)
        return _strassen_steps(lambda t: _mm(_bf(o_terms[t]), _bf(wo[layer, p, t])), emit)

    def a_body(i, _):
        seg, p = i // NP, i % NP
        slot = seg % 2
        zero = i // (NSEG * NP)
        live = {}

        def qk_steps(is_k):
            def emit(rh, t, y):
                ph = _phi(y)
                if is_k:
                    zs = jnp.sum(ph.reshape(-1, 8, 128), axis=0)
                    live["z", t] = live["z", t] + zs if ("z", t) in live else zs
                a, b = (k_a, pk_a) if is_k else (qs_a, pq_a)
                y, ph = _pack_all([y if is_k else y * QSCALE, ph])
                for j in range(2):
                    a[t, prows(2 * j + rh)] = y[j * 64:(j + 1) * 64]
                    b[t, prows(2 * j + rh)] = ph[j * 64:(j + 1) * 64]
            return _strassen_steps(lambda n: _mm(_bf(xs[slot, n]), _bf(wa_qk[2 * p + is_k, n])), emit)

        def v_steps():
            def emit(rh, nh, y):
                y = _pack(y)
                for j in range(2):
                    vt_a[nh, :, rows(2 * j + rh)] = y[:, j * C:(j + 1) * C]
            return _strassen_steps(lambda n: _mm(_bf(wa_v[p, n]), _bf(xs[slot, n]), NT), emit)

        def scores(t, c):
            nk = (c + 1) * C
            qj = qs_a[t, prows(c)]
            qbd = jnp.concatenate([jnp.where(lane64 // DH == h, qj, jnp.zeros_like(qj)) for h in range(4)], axis=0)
            st = _mm(_bf(k_a[t, :nk // 2]), _bf(qbd), NT)
            for h in range(4):
                sh = st[:, h * 128:(h + 1) * 128]
                sd = jnp.where(causal, sh[nk - C:], -1e30)
                sh = sd if c == 0 else jnp.concatenate([sh[:nk - C], sd], axis=0)
                live["max", t, c, h] = jnp.max(sh, axis=0, keepdims=True)
                sc[2 * c + t][h, :nk] = sh
            return st

        def mem_read(t):
            g = 2 * p + t
            zs = jnp.sum(z_s[g], axis=0, keepdims=True)
            zrows = jnp.where(lane16 // DH == row16, jnp.broadcast_to(zs, (16, 128)), 0.0)
            maug = jnp.concatenate([mt_s[g], zrows], axis=0).astype(BF16)
            live["m", t] = _mm(maug, _bf(pq_a[t]), NT)
            return live["m", t]

        def mem_write(t):
            g = 2 * p + t
            y = _mm(_bf(vt_a[t]), _bf(pk_a[t]))
            mt_s[g] += jnp.where(same_head, y, 0.0)
            z_s[g] += live.pop(("z", t))
            return y

        def mix(t, heads, y):
            for c in sorted({c for c, _ in heads}):
                sc[2 * c + t][4 + zero, :8] = y
            for c, h in heads:
                nk = (c + 1) * C
                e = jnp.exp2(sc[2 * c + t][h, :nk] - live.pop(("max", t, c, h)))
                l = jnp.sum(e, axis=0, keepdims=True)
                ot = _mm(_bf(vt_a[t, h * DH // 2:(h + 1) * DH // 2, :nk]), e.astype(BF16))
                numt = live["m", t][:, c * C:(c + 1) * C]
                gate = gate_s[pl.ds((2 * p + t) * 4 + h, 1), :]
                den = numt[128 + h:128 + h + 1] + 1e-6
                live["o", t, c, h] = ot * ((1.0 - gate) / l) + numt[h * DH:(h + 1) * DH] * (gate / den)
                if all(("o", t, c, k) in live for k in range(4)):
                    live["o", t, c] = jnp.concatenate([live.pop(("o", t, c, k)) for k in range(4)], axis=0).T
                quad = [("o", k, c // 2 * 2 + r) for r in range(2) for k in range(2)]
                if all(k in live for k in quad):
                    live["ot", c // 2] = _pack_all(_x_terms(*[live.pop(k) for k in quad]))

        def stage(t, j, v):
            x_new[t, pl.ds(j * 8, 8)] = v

        def store_x(t, y):
            x_new[7 + zero, :8, :128] = lax.bitcast_convert_type(y, U32)
            xs[1 - slot, t, pl.ds(pl.multiple_of(p * 32, 32), 32)] = x_new[t, :32]

        ln = ln_steps((seg + 1) % NSEG, p * 64, 64, stage, zero)
        out = out_steps((seg + NSEG - 1) % NSEG, jnp.where(seg == 0, 1, 0), os_.at[1 - slot], p)
        v, k = v_steps(), qk_steps(1)
        _weave(v + qk_steps(0), ln)
        _weave(k + [P(mem_read, 0)])
        jobs = ([(t, [(3, h)]) for t in range(2) for h in range(4)]
                + [(t, [(2, h), (0, h)]) for t in range(2) for h in range(4)]
                + [(t, [(1, h), (1, h + 1)]) for t in range(2) for h in (0, 2)])
        sx = [P(store_x, t) for t in range(7)]
        fill = [P(scores, 0, 3), P(mem_read, 1), P(scores, 1, 3), out[0], P(scores, 0, 2), P(scores, 0, 0), out[1],
                P(scores, 1, 2), P(scores, 1, 0), out[2], P(scores, 0, 1), P(scores, 1, 1), out[3], out[4],
                P(mem_write, 0), out[5], out[6], P(mem_write, 1)]
        njobs = [0, 0, 2, 2, 2, 1, 1, 2, 1, 2, 2, 2, 1, 1, 1, 0, 0, 0]
        y = None
        for f, n in zip(fill, njobs):
            y0, y = y, f()
            for j in range(n):
                t, heads = jobs.pop(0)
                mix(t, heads, y0[-8:, :128] if j == 0 else y[:8, :128])
            if sx and f in out:
                sx.pop()(y[:8])
        for c in (1, 0):
            for n, v in enumerate(live.pop(("ot", c))):
                os_[slot, n, prows(c), _tile(p)] = v

    def b_body(rep, seg, _):
        zero = seg // NSEG

        def proj_steps(t, p):
            def emit(rh, nh, y):
                for i in range(2):
                    c = 2 * i + rh
                    yi = y[i * C:(i + 1) * C]
                    dst, g = (q_b, k_b, v_b)[t], 2 * p + nh
                    if t == 0:
                        dst[g, rows(c)] = yi * QSCALE
                        continue
                    if c == NC - 1:
                        dst[g, :HALO] = dst[g, L:]
                    dst[g, pl.ds(HALO + c * C, C)] = yi
            return _strassen_steps(lambda n: _mm(_bf(xs[0, n]), _bf(wb[t * NP + p, n]), NT), emit)

        def shifted(ref, g, r0, w, n):
            return ref[g, pl.ds(r0 + HALO - DIL * w, n)]

        def logit_steps(p):
            def f(r0, y):
                q_b[NG + zero, :8] = y
                for w in range(W):
                    acc = None if p == 0 else lg_b[w, r0:r0 + RB]
                    for g in (2 * p, 2 * p + 1):
                        t = q_b[g, r0:r0 + RB, :] * shifted(k_b, g, r0, w, RB)
                        acc = t if acc is None else acc + t
                    lg_b[w, r0:r0 + RB] = acc
            return [P(f, r0) for r0 in range(0, L, RB)]

        def softmax_steps():
            def f(r0, y):
                lg_b[W + zero, :8] = y
                lg = []
                for w in range(W):
                    acc = lg_b[w, r0:r0 + RB]
                    acc = acc + pltpu.roll(acc, 64, 1)
                    acc = acc + pltpu.roll(acc, 32, 1)
                    if w and r0 < DIL * w:
                        pos = seg * L + r0 + lax.broadcasted_iota(jnp.int32, (RB, 128), 0)
                        acc = jnp.where(pos >= DIL * w, acc, -1e9 * LOG2E)
                    lg.append(acc)
                m = functools.reduce(jnp.maximum, lg)
                e = [jnp.exp2(t - m) for t in lg]
                inv = 1.0 / functools.reduce(jnp.add, e)
                for w in range(W):
                    p_b[w, r0:r0 + RB] = e[w] * inv
            return [P(f, r0) for r0 in range(0, L, RB)]

        def mix_steps(p):
            def f(r, y):
                p_b[W + zero, :8] = y
                quad = []
                for r0 in (r // C * 2 * C + r % C, r // C * 2 * C + r % C + C):
                    pw = [p_b[w, r0:r0 + 16] for w in range(W)]
                    for g in (2 * p, 2 * p + 1):
                        quad.append(functools.reduce(jnp.add, [pw[w] * shifted(v_b, g, r0, w, 16) for w in range(W)]))
                for n, v in enumerate(_pack_all(_x_terms(*quad))):
                    os_[1, n, pl.ds(r // 2, 8), _tile(p)] = v
            return [P(f, r) for r in range(0, L // 2, 16)]

        prev = (seg + NSEG - 1) % NSEG
        def stage(t, j, v):
            x_new[t, pl.ds(j * 8, 8)] = v

        def copy_o(t, j, y):
            os_[zero, 0, :8, :128] = lax.bitcast_convert_type(y, U32)
            o_cur[t, j * 32:(j + 1) * 32] = os_[1, t, j * 32:(j + 1) * 32]

        def copy_x(t, j, y):
            x_new[7 + zero, :8, :128] = lax.bitcast_convert_type(y, U32)
            xs[0, t, j * 32:(j + 1) * 32] = x_new[t, j * 32:(j + 1) * 32]

        out = [out_steps(prev, jnp.where(seg == 0, 0, 1), o_cur, p, True) for p in range(NP)]
        ln = ln_steps((seg + 1) % NSEG, 0, L // 2, stage, zero)
        cp = [P(copy_o, t, j) for t in range(7) for j in range(4)]
        _weave(proj_steps(0, 0) + proj_steps(1, 0), ln[:10])
        _weave(proj_steps(0, 1) + proj_steps(1, 1), logit_steps(0), ln[10:])
        _weave(proj_steps(0, 2) + proj_steps(1, 2), logit_steps(1), cp[:14])
        _weave(proj_steps(0, 3) + proj_steps(1, 3), logit_steps(2), cp[14:])
        _weave(proj_steps(2, 0), logit_steps(3))
        _weave(out[0] + out[1] + proj_steps(2, 1)[:0], softmax_steps())
        for p in range(1, NP):
            _weave(proj_steps(2, p), mix_steps(p - 1))
        _weave(out[2], mix_steps(NP - 1))
        _weave(out[3], [P(copy_x, t, j) for t in range(7) for j in range(4)])

        @pl.when(jnp.logical_and(rep == 1, seg > 0))
        def _():
            out_copy(prev).start()

    def layer_pair(rep, _):
        mt_s[...] = jnp.zeros(mt_s.shape, F32)
        z_s[...] = jnp.zeros(z_s.shape, F32)
        k_b[:, L:] = jnp.zeros((NG, HALO, 128), F32)
        v_b[:, L:] = jnp.zeros((NG, HALO, 128), F32)
        lax.fori_loop(0, NSEG * NP, a_body, None)
        lax.fori_loop(0, NSEG, P(b_body, rep), None)
    lax.fori_loop(0, 2, layer_pair, None)

    def last(p, _):
        _weave(out_steps(NSEG - 1, 1, os_.at[1], p, True))
    lax.fori_loop(0, NP, last, None)
    out_copy(NSEG - 1).start()
    for s in range(NSEG):
        out_copy(s).wait()


@jax.jit
def pallas_interleave_layers__memory_aug_infini_attn__sliding_local_dilated__prompt_kernel(
        A_x, A_wq, A_wk, A_wv, A_wo, A_beta, B_x, B_wqkv, B_wo):
    del B_x
    hbm = pl.BlockSpec(memory_space=pl.ANY)
    V = pltpu.VMEM
    scratch = [
        V((S, D), BF16), V((3, D, D), BF16), V((D, 3 * D), BF16), V((2, D, D), BF16),
        V((3, H * (DH + 1), 128), U32),
        V((NG, 7, KH // 2, 128), U32), V((NP, 7, 64, KH), U32), V((NG + NP, 7, 64, KH), U32),
        V((2, NP, 7, KH // 2, 128), U32),
        V((H, 128), F32), V((NSEG + 1, L, D), F32), V((8, L // 4, KH), U32), V((2, 7, L // 4, KH), U32), V((2, 7, L // 4, KH), U32),
        V((NG, 128, 128), F32), V((NG, 8, 128), F32),
        V((2, L // 2, 128), U32), V((2, L // 2, 128), U32), V((2, L // 2, 128), U32), V((2, L // 2, 128), U32),
        V((2, 64, L), U32),
        V((NG + 1, L, 128), F32), V((NG, L + HALO, 128), F32), V((NG, L + HALO, 128), F32), V((W + 1, L, 128), F32),
        V((W + 1, L, 128), F32), V((7, L // 4, KH), U32),
        pltpu.SemaphoreType.DMA((11,)),
    ] + [V((5, (c + 1) * C, 128), F32) for c in range(NC) for _ in range(2)]
    return pl.pallas_call(
        _kernel,
        in_specs=[hbm, pl.BlockSpec(memory_space=pltpu.VMEM), hbm, hbm, hbm, hbm, hbm, hbm],
        out_specs=hbm,
        out_shape=jax.ShapeDtypeStruct(A_x.shape, A_x.dtype),
        scratch_shapes=scratch,
        compiler_params=pltpu.CompilerParams(
            vmem_limit_bytes=110 * 2 ** 20,
            flags={os.environ['KCFG_FLAG']: True} if 'KCFG_FLAG' in os.environ else None),
        name="interleaved_attn",
    )(A_x, A_beta, A_wq, A_wk, A_wv, A_wo, B_wqkv, B_wo)
```

```python
import functools
import math
import os

import jax
import jax.numpy as jnp
import numpy as np
from jax import lax
from jax.experimental import pallas as pl
from jax.experimental.pallas import tpu as pltpu

S, D, H, DH = 2048, 1024, 32, 32
L = 512
NSEG = S // L
NG = D // 128
NP = NG // 2
C = 128
NC = L // C
KH = D // 2
W, DIL = 8, 2
HALO = 16
LOG2E = math.log2(math.e)
QSCALE = DH ** -0.5 * LOG2E
F32, BF16, U32 = jnp.float32, jnp.bfloat16, jnp.uint32
NN = (((1,), (0,)), ((), ()))
NT = (((1,), (1,)), ((), ()))
cfg = lambda k, d: int(os.environ.get("KCFG_" + k, d))
RB = cfg("RB", 8)
P = functools.partial


def _mm(a, b, dims=NN):
    return lax.dot_general(a, b, dims, preferred_element_type=F32)


def _pack(*xs):
    return pltpu.bitcast(jnp.concatenate(xs, axis=1).astype(BF16), U32)


def _bf(x):
    return pltpu.bitcast(x, BF16)


def _bits(x):
    return lax.bitcast_convert_type(x.astype(F32), U32)


def _join(lo, hi):
    return (_bits(lo) >> 16) | _bits(hi)


def _split(p):
    return (lax.bitcast_convert_type(p << 16, F32),
            lax.bitcast_convert_type(p & np.uint32(0xFFFF0000), F32))


def _layernorm(x):
    m = jnp.mean(x, axis=-1, keepdims=True)
    xc = x - m
    v = jnp.mean(xc * xc, axis=-1, keepdims=True)
    return xc * lax.rsqrt(v + 1e-5)


def _phi(t):
    return jnp.where(t > 0, t + 1.0, jnp.exp(t))


def _x_terms(x11, x12, x21, x22):
    return (x11 + x22, x21 + x22, x11, x22, x11 + x12, x21 - x11, x12 - x22)


def _w_terms(w11, w12, w21, w22):
    return (w11 + w22, w11, w12 - w22, w21 - w11, w22, w11 + w12, w21 + w22)


def _strassen_steps(prod, emit):
    m = {}

    def step(i):
        y = prod(i)
        if i == 1:
            m[1] = y
        elif i == 3:
            m[3] = y
            emit(1, 0, m[1] + y)
        elif i == 4:
            m[4] = y
            m["a"] = m.pop(3) - y
        elif i == 2:
            emit(0, 1, y + m.pop(4))
            m["b"] = y - m.pop(1)
        elif i == 0:
            m["a"] += y
            m["b"] += y
        elif i == 6:
            emit(0, 0, m.pop("a") + y)
        else:
            emit(1, 1, m.pop("b") + y)
        return y
    return [P(step, i) for i in (1, 3, 4, 2, 0, 6, 5)]


def _weave(mxu, *side):
    after = [[] for _ in mxu]
    for steps in side:
        for i, f in enumerate(steps):
            pos = (i + 0.5) / len(steps) * len(mxu)
            after[int(pos)].append((pos % 1.0, f))
    for f, todo in zip(mxu, after):
        y = f()
        for frac, g in sorted(todo, key=lambda t: t[0]):
            r = int(frac * (y.shape[0] // 8)) * 8
            g(y[r:r + 8, :128])


def _ds(start, size, align=None):
    if not isinstance(start, int):
        start = pl.multiple_of(start, align or size)
    return pl.ds(start, size)


def _tile(g, n=1):
    return _ds(g * 128, n * 128, 128)


def _kernel(x_h, beta_ref, awq_h, awk_h, awv_h, awo_h, bwqkv_h, bwo_h, out_h,
            io_s, raw_q, raw_k, raw_v, raw_ao, raw_bo, raw_b, tmp_s, wa_q, wa_k, wa_v, wb, wo,
            gate_s, x_s, x_new, xs, os_, o_cur, mt_s, z_s, q_a, k_a, vt_a,
            q_b, k_b, v_b, lg_b, p_b, sc, sem_x, sem_o, sem_w):
    def x_copy(j):
        r = _ds(j * (L // 2), L // 2)
        return pltpu.make_async_copy(x_h.at[0, r], io_s.at[r], sem_x.at[j])

    def out_copy(s):
        return pltpu.make_async_copy(io_s.at[_ds(s * L, L)], out_h.at[0, _ds(s * L, L)], sem_o.at[s])

    def last_copy(p):
        r, c = pl.ds(S - L, L), _tile(2 * p, 2)
        return pltpu.make_async_copy(io_s.at[r, c], out_h.at[0, r, c], sem_o.at[NSEG - 1 + p])

    def w_copy(i, p):
        src, dst = ((awv_h, raw_v), (awk_h, raw_k), (awq_h, raw_q), (awo_h, raw_ao), (bwo_h, raw_bo))[i]
        return pltpu.make_async_copy(src.at[:, _tile(2 * p, 2)], dst.at[p], sem_w.at[i * NP + p])

    def b_copy(t):
        return pltpu.make_async_copy(bwqkv_h.at[:, _ds(t * D, D)], raw_b.at[t], sem_w.at[5 * NP + t])

    def pace(ref, idx, y):
        if y is not None:
            if ref.dtype == BF16:
                y = jnp.concatenate([y, y], axis=0)
            y = _bits(y) if ref.dtype == U32 else y.astype(ref.dtype)
            ref[(*idx, slice(0, y.shape[0]), slice(0, 128))] = y

    def ln_steps(s, r0, n, dst, d0, zero):
        def f(i, y):
            pace(x_s, (NSEG + zero,), y)
            r = r0 + i * 16
            a = (r // C) * (2 * C) + r % C
            y1 = _layernorm(x_s[s, _ds(a, 16)])
            y2 = _layernorm(x_s[s, _ds(a + C, 16)])
            for t, v in enumerate(_x_terms(y1[:, :KH], y1[:, KH:], y2[:, :KH], y2[:, KH:])):
                dst.at[t][_ds(d0 + i * 8, 8)] = _pack(v)
        return [P(f, i) for i in range(n // 16)]

    def widen(s, a, n):
        x_s[s, _ds(a, n)] = io_s[_ds(s * L + a, n)].astype(F32)

    def prep_qk_steps(raw, dst, p, zero, n=32):
        def f(k0, y):
            pace(raw, (NP + zero,), y)
            w1, w2 = raw[p, k0:k0 + n].astype(F32), raw[p, KH + k0:KH + k0 + n].astype(F32)
            dst.at[p][k0 // 2:(k0 + n) // 2] = _pack(*_w_terms(w1[:, :128], w1[:, 128:], w2[:, :128], w2[:, 128:]))
        return [P(f, k0) for k0 in range(0, KH, n)]

    def prep_v_steps(p, zero):
        def f(kt, y):
            pace(raw_v, (NP + zero,), y)
            lo, hi = _split(_join(raw_v[p, _tile(kt)], raw_v[p, _tile(NP + kt)]).T)
            wa_v.at[p, kt][...] = _pack(*_w_terms(lo[:128], lo[128:], hi[:128], hi[128:]))
        return [P(f, kt) for kt in range(NP)]

    def prep_ao_steps(p, zero, n=32):
        def f(kp, k0, y):
            pace(raw_ao, (NP + zero,), y)
            w1 = raw_ao[p, pl.ds(kp * 256 + k0, n)].astype(F32)
            w2 = raw_ao[p, pl.ds(kp * 256 + 128 + k0, n)].astype(F32)
            wo.at[0, p][pl.ds(kp * 64 + k0 // 2, n // 2)] = _pack(
                *_w_terms(w1[:, :128], w1[:, 128:], w2[:, :128], w2[:, 128:]))
        return [P(f, kp, k0) for kp in range(NP) for k0 in range(0, 128, n)]

    def spread(g, v):
        for h in range(4):
            tmp_s[0, pl.ds((4 * g + h) * (DH + 1), DH)] = v[h * DH:(h + 1) * DH]

    def gather(g, d):
        return tmp_s[0, pl.ds(4 * g + d, H, stride=DH + 1)]

    def prep_bo_steps(p, zero):
        def f(g, y):
            pace(raw_bo, (NP + zero,), y)
            w = raw_bo[p, _tile(g)]
            spread(g, _join(w[:, :128], w[:, 128:]))

        def h(kp, d, y):
            pace(tmp_s, (1 + zero,), y)
            (w11, w12), (w21, w22) = _split(gather(2 * kp, d)), _split(gather(2 * kp + 1, d))
            wo.at[1, p][pl.ds(kp * 64 + d * 16, 16)] = _pack(*_w_terms(w11, w12, w21, w22))
        return [P(f, g) for g in range(NG)] + [P(h, kp, d) for kp in range(NP) for d in range(4)]

    def prep_b_steps(t, kt, zero):
        def f(g, y):
            pace(raw_b, (3 + zero,), y)
            spread(g, _join(raw_b[t, _tile(kt), _tile(g)], raw_b[t, _tile(NP + kt), _tile(g)]).T)

        def h(p, d, y):
            pace(tmp_s, (1 + zero,), y)
            (w11, w21), (w12, w22) = _split(gather(2 * p, d)), _split(gather(2 * p + 1, d))
            wb.at[t * NP + p, kt][pl.ds(d * 16, 16)] = _pack(*_w_terms(w11, w12, w21, w22))
        return [P(f, g) for g in range(NG)] + [P(h, p, d) for p in range(NP) for d in range(4)]

    def k_tiles(ref, n):
        return _bf(jnp.concatenate([ref[kt, :, _tile(n)] for kt in range(NP)], axis=1))

    def rows(c):
        return pl.ds(c * C, C)

    def prows(c):
        return pl.ds(c * C // 2, C // 2)

    def out_steps(s, layer, o_terms, p, final=False):
        def emit(rh, nh, y):
            for i in range(2):
                c = 2 * i + rh
                x = x_s[s, rows(c), _tile(2 * p + nh)] + y[i * C:(i + 1) * C]
                x_s[s, rows(c), _tile(2 * p + nh)] = x
                if final:
                    io_s[_ds(s * L + c * C, C), _tile(2 * p + nh)] = x.astype(io_s.dtype)
        return _strassen_steps(lambda n: _mm(k_tiles(o_terms, n), _bf(wo[layer, p, :, _tile(n)])), emit)

    lane = lax.broadcasted_iota(jnp.int32, (128, 128), 1)
    row = lax.broadcasted_iota(jnp.int32, (128, 128), 0)
    same_head = (lane // DH) == (row // DH)
    lane64 = lax.broadcasted_iota(jnp.int32, (64, 128), 1)
    row64 = lax.broadcasted_iota(jnp.int32, (64, 128), 0)
    lane1 = lax.broadcasted_iota(jnp.int32, (1, 128), 1)
    late = (lane1 < 64, lane1 >= 64)

    def swap_even(y):
        return jnp.where(lane // DH % 2 == 0, jnp.concatenate([y[64:], y[:64]], axis=0), y)
    lane16 = lax.broadcasted_iota(jnp.int32, (16, 128), 1)
    row16 = lax.broadcasted_iota(jnp.int32, (16, 128), 0)

    def a_body(first, i, _):
        seg, p = (0, i) if first else (i // NP, i % NP)
        slot = seg % 2
        zero = i // (NSEG * NP)
        live = {}

        def qk_steps(is_k):
            def emit(rh, t, y):
                if not is_k:
                    y = jnp.concatenate([swap_even(y[:C]), swap_even(y[C:])], axis=0)
                ph = _phi(y)
                if is_k:
                    zs = jnp.sum(ph.reshape(-1, 8, 128), axis=0)
                    live["z", t] = live["z", t] + zs if ("z", t) in live else zs
                dst, y = (k_a, y) if is_k else (q_a, y * QSCALE)
                for j in range(2):
                    dst.at[t][prows(2 * j + rh)] = _pack(y[j * C:(j + 1) * C], ph[j * C:(j + 1) * C])
            w = wa_k if is_k else wa_q
            return _strassen_steps(lambda n: _mm(_bf(xs[slot, n]), _bf(w[p, :, _tile(n)])), emit)

        def v_steps():
            def emit(rh, t, y):
                vt_a.at[t][:, _tile(2 * rh, 2)] = _pack(y)
            return _strassen_steps(lambda n: _mm(k_tiles(wa_v.at[p], n), _bf(xs[slot, n]), NT), emit)

        def vt(t, r, nc):
            return _bf(jnp.concatenate([vt_a[t, r, _tile(c % 2 * 2 + c // 2)] for c in range(nc)], axis=1))

        def scores(t, c):
            nk = c * C + 64
            qj = q_a[t, prows(c), :128]
            qbd = jnp.concatenate([jnp.where(lane64 // DH == h, qj, jnp.zeros_like(qj)) for h in range(4)], axis=0)
            st = _mm(_bf(k_a[t, :nk // 2, :128]), _bf(qbd), NT)
            for h in range(4):
                sh = st[:, h * 128:(h + 1) * 128]
                sd = jnp.where(row64 <= (lane64 if h % 2 else lane64 ^ 64), sh[nk - 64:], -1e30)
                sh = sd if c == 0 else jnp.concatenate([sh[:nk - 64], sd], axis=0)
                live["max", t, c, h] = jnp.max(sh, axis=0, keepdims=True)
                sc[2 * c + t][h] = sh
            for j in range(2):
                se = live.pop(("edge", t, c, j))
                me = jnp.max(se, axis=0, keepdims=True)
                for n in range(2):
                    m = live["max", t, c, 2 * j + n]
                    live["max", t, c, 2 * j + n] = jnp.where(late[n], jnp.maximum(m, me), m)
                live["edge", t, c, j] = se - jnp.where(late[0], live["max", t, c, 2 * j], live["max", t, c, 2 * j + 1])
            return st

        def edge_scores(t, rh):
            for c in (rh, rh + 2):
                qj = q_a[t, prows(c), :128]
                qbd = jnp.concatenate([jnp.where(lane64 // DH == 2 * j + row64 // 32, qj, jnp.zeros_like(qj))
                                       for j in range(2)], axis=0)
                st = _mm(_bf(k_a[t, pl.ds(c * 64 + 32, 32), :128]), _bf(qbd), NT)
                for j in range(2):
                    live["edge", t, c, j] = jnp.where(row64 <= lane64 % 64, st[:, j * 128:(j + 1) * 128], -1e30)
            return st

        def mem_read(t):
            g = 2 * p + t
            zs = jnp.sum(z_s[g], axis=0, keepdims=True)
            zrows = jnp.where(lane16 // DH == row16, jnp.broadcast_to(zs, (16, 128)), 0.0)
            maug = jnp.concatenate([mt_s[g], zrows], axis=0).astype(BF16)
            live["m", t] = _mm(maug, _bf(q_a[t, :, 128:]), NT)
            return live["m", t]

        def mem_write(t):
            g = 2 * p + t
            y = _mm(vt(t, slice(None), NC), _bf(k_a[t, :, 128:]))
            mt_s[g] += jnp.where(same_head, y, 0.0)
            z_s[g] += live.pop(("z", t))
            return y

        def mix(heads, ys):
            for t, c, h in heads:
                m = live.pop(("max", t, c, h))
                e = []
                for r in range(0, c * C + 64, 64):
                    y = ys.pop(0)
                    if r % cfg("PG", 128) == 0:
                        pace(sc[2 * c + t], (4 + zero,), y)
                    e.append(jnp.exp2(sc[2 * c + t][h, r:r + 64] - m))
                ys.pop(0)
                if h % 2 == 0:
                    live["edge", t, c, h // 2] = jnp.exp2(live["edge", t, c, h // 2])
                e = jnp.concatenate(e + [jnp.where(late[h % 2], live["edge", t, c, h // 2], 0.0)], axis=0)
                gate = gate_s[pl.ds((2 * p + t) * 4 + h, 1), :]
                live["o", t, c, h] = (_mm(vt(t, pl.ds(h * DH // 2, DH // 2), c + 1), e.astype(BF16))
                                      * ((1.0 - gate) / jnp.sum(e, axis=0, keepdims=True)))

        def finish():
            for t in range(2):
                for c in range(NC):
                    if ("m", t) in live and all(("o", t, c, h) in live for h in range(4)):
                        numt = live["m", t][:, c * C:(c + 1) * C]
                        outs = []
                        for h in range(4):
                            gate = gate_s[pl.ds((2 * p + t) * 4 + h, 1), :]
                            den = numt[128 + h:128 + h + 1] + 1e-6
                            outs.append(live.pop(("o", t, c, h)) + numt[h * DH:(h + 1) * DH] * (gate / den))
                        live["o", t, c] = swap_even(jnp.concatenate(outs, axis=0).T)

        def store_x(t, y):
            pace(x_new, (7 + zero,), y)
            xs[1 - slot, t, _ds(p * 32, 32)] = x_new[t, :32]

        ln = ln_steps((seg + 1) % NSEG, p * 64, 64, x_new, 0, zero)
        v, q, k = v_steps(), qk_steps(0), qk_steps(1)
        sx = [P(store_x, t) for t in range(7)]
        jobs = ([[(0, 3, h)] for h in range(4)] + [[(0, 1, h), (0, 1, h + 1)] for h in (0, 2)]
                + [[(t, 2, h), (t, 0, h)] for t in (1, 0) for h in range(4)]
                + [[(1, 3, h)] for h in range(4)] + [[(1, 1, h), (1, 1, h + 1)] for h in (0, 2)])
        E, Q, R, U = edge_scores, scores, mem_read, mem_write
        if first:
            nxt = jnp.minimum(p + 1, NP - 1)

            def wait(cond, copy, y=None):
                pl.when(cond)(lambda: copy().wait())

            def widen_step(s, j, y):
                io_s[_ds(zero * 16, 16), :128] = jnp.concatenate([y, y], axis=0).astype(BF16)
                widen(s, p // 2 * 256 + p % 2 * 64 + j % 2 * C + j // 2 * 16, 16)

            @pl.when(p == 0)
            def _():
                w_copy(0, 1).start()
                x_copy(2).start()
                w_copy(3, 0).start()
            w_copy(1, p).wait()
            w_copy(2, p).wait()
            _weave(v[:6], prep_qk_steps(raw_k, wa_k, p, zero) + prep_qk_steps(raw_q, wa_q, p, zero))
            _weave(v[6:])
            wait(p < NP - 1, lambda: w_copy(0, nxt))
            wait(p % 2 == 0, lambda: x_copy(2 + p // 2))

            @pl.when(p < NP - 1)
            def _():
                for n in range(1, 4):
                    w_copy(n, nxt).start()
            pl.when(p < NP - 2)(lambda: w_copy(0, jnp.minimum(p + 2, NP - 1)).start())
            w_copy(4, p).start()
            pl.when(p == 0)(lambda: x_copy(3).start())
            x_copy(4 + p).start()
            pl.when(p > 0)(lambda: b_copy(jnp.maximum(p - 1, 0)).start())
            w_copy(3, p).wait()
            wd = [P(widen_step, 1, j) for j in range(8)]
            _weave(k + q[:3], prep_v_steps(nxt, zero), prep_ao_steps(p, zero),
                   [f for j in range(4) for f in wd[2 * j:2 * j + 2] + ln[j:j + 1]])
            jobs = jobs[:10] + jobs[14:] + jobs[10:14]
            fill = [(P(E, 0, 1), 0), (P(Q, 0, 3), 0), (q[3], 0), (P(Q, 0, 1), 1), (q[4], 2), (P(E, 1, 0), 0),
                    (P(Q, 1, 2), 2), (P(Q, 1, 0), 0), (q[5], 1), (q[6], 2), (P(R, 0), 1), (P(E, 1, 1), 0),
                    (P(Q, 1, 3), 1), (P(Q, 1, 1), 0), (P(E, 0, 0), 1), (P(Q, 0, 2), 2), (P(Q, 0, 0), 1),
                    (P(R, 1), 2), (P(U, 0), 2), (P(U, 1), 2)]
            side = [[lambda y: None] * 10 + sx + [lambda y: None] * 3]
        else:
            out = out_steps((seg + NSEG - 1) % NSEG, jnp.where(seg == 0, 1, 0), os_.at[1 - slot], p)
            prep = prep_b_steps(jnp.maximum(seg - 1, 0), p, zero) + prep_bo_steps(p, zero)
            _weave(k + v + q[:3], ln, prep)
            fill = [(P(E, 0, 1), 0), (P(Q, 0, 3), 0), (q[3], 0), (P(Q, 0, 1), 1), (q[4], 1), (P(E, 1, 0), 0),
                    (P(Q, 1, 2), 2), (P(Q, 1, 0), 0), (q[5], 1), (q[6], 1), (P(R, 0), 1), (P(E, 0, 0), 0),
                    (P(Q, 0, 2), 2), (P(Q, 0, 0), 0), (P(R, 1), 1), (P(E, 1, 1), 0), (P(Q, 1, 3), 2),
                    (P(Q, 1, 1), 1), (out[0], 1), (out[1], 1), (out[2], 1), (out[3], 1), (P(U, 0), 1),
                    (out[4], 1), (P(U, 1), 1), (out[5], 0), (out[6], 0)]
            side = [[lambda y: None] * 7 + sx]

        LAG = cfg("LAG", 160)
        hist = []

        def fill_step(f, n):
            y = f()
            hist.extend(y[r:r + 8, :128] for r in range(0, y.shape[0], 8))
            for j in range(n):
                mix(jobs.pop(0), [hist[max(0, len(hist) - (LAG + cfg("GAP", 24) * (8 * (n - j) - u)) // 8)]
                                  for u in range(8)])
            finish()
            return y
        _weave([P(fill_step, f, n) for f, n in fill], *side)
        assert not jobs
        for j in (1, 0):
            os_.at[slot, p][prows(j)] = _pack(*_x_terms(*[live.pop(("o", t, 2 * j + r)) for r in range(2) for t in range(2)]))

    def b_body(rep, seg, _):
        zero = seg // NSEG

        def proj_steps(t, p):
            def emit(rh, nh, y):
                for i in range(2):
                    c = 2 * i + rh
                    yi = y[i * C:(i + 1) * C]
                    if t == 0:
                        q_b[p][nh, rows(c)] = yi * QSCALE
                        continue
                    dst, g = (k_b, v_b)[t - 1], 2 * p + nh
                    if c == NC - 1:
                        dst[g, :HALO] = dst[g, L:]
                    dst[g, pl.ds(HALO + c * C, C)] = yi
            return _strassen_steps(lambda n: _mm(_bf(xs[0, n]), k_tiles(wb.at[t * NP + p], n), NT), emit)

        def shifted(ref, g, r0, w, n):
            return ref[g, pl.ds(r0 + HALO - DIL * w, n)]

        def logit_steps(p):
            def f(r0, y):
                pace(q_b[p], (2 + zero,), y)
                lg = []
                for w in range(W):
                    acc = None if p == 0 else lg_b[w, r0:r0 + 8]
                    for n in range(2):
                        t = q_b[p][n, r0:r0 + 8, :] * shifted(k_b, 2 * p + n, r0, w, 8)
                        acc = t if acc is None else acc + t
                    if p < NP - 1:
                        lg_b[w, r0:r0 + 8] = acc
                        continue
                    acc = acc + pltpu.roll(acc, 64, 1)
                    acc = acc + pltpu.roll(acc, 32, 1)
                    if w and r0 < DIL * w:
                        pos = seg * L + r0 + lax.broadcasted_iota(jnp.int32, (8, 128), 0)
                        acc = jnp.where(pos >= DIL * w, acc, -1e9 * LOG2E)
                    lg.append(acc)
                if lg:
                    m = functools.reduce(jnp.maximum, lg)
                    e = [jnp.exp2(t - m) for t in lg]
                    inv = 1.0 / functools.reduce(jnp.add, e)
                    for w in range(W):
                        p_b[w, r0:r0 + 8] = e[w] * inv
            return [P(f, r0) for r0 in range(0, L, 8)]

        def mix_steps(p):
            part = []

            def f(r, j, y):
                pace(p_b, (W + zero,), y)
                r0 = r // C * 2 * C + r % C + j // 2 * C + j % 2 * 8
                pw = [p_b[w, r0:r0 + 8] for w in range(W)]
                part.append([functools.reduce(jnp.add, [pw[w] * shifted(v_b, g, r0, w, 8) for w in range(W)])
                             for g in (2 * p, 2 * p + 1)])
                if j == 3:
                    quad = [jnp.concatenate([part[2 * a][b], part[2 * a + 1][b]], axis=0)
                            for a in range(2) for b in range(2)]
                    part.clear()
                    os_.at[1, p][pl.ds(r // 2, 8)] = _pack(*_x_terms(*quad))
            return [P(f, r, j) for r in range(0, L // 2, 16) for j in range(4)]

        def copy_o(p, j, y):
            pace(os_, (zero, 0), y)
            o_cur[p, j * 16:(j + 1) * 16] = os_[1, p, j * 16:(j + 1) * 16]

        def copy_x(t, j, y):
            pace(x_new, (7 + zero,), y)
            xs[0, t, j * 16:(j + 1) * 16] = x_new[t, j * 16:(j + 1) * 16]

        prev = (seg + NSEG - 1) % NSEG
        out = [out_steps(prev, jnp.where(seg == 0, 0, 1), o_cur, p, True) for p in range(NP)]
        ln = ln_steps((seg + 1) % NSEG, 0, L // 2, x_new, 0, zero)
        cp = [P(copy_o, p, j) for p in range(NP) for j in range(8)]
        _weave(proj_steps(2, 0) + proj_steps(0, 0) + proj_steps(1, 0), ln)
        _weave(proj_steps(0, 1) + proj_steps(1, 1), logit_steps(0), cp[:12])
        _weave(proj_steps(0, 2) + proj_steps(1, 2), logit_steps(1), cp[12:22])
        _weave(proj_steps(0, 3) + proj_steps(1, 3), logit_steps(2), cp[22:])
        rest = proj_steps(2, 1) + proj_steps(2, 2) + proj_steps(2, 3) + out[0] + out[1] + out[2] + out[3]
        n1, n2 = cfg("N1", 17), cfg("N2", 19)
        _weave(rest[:n1], logit_steps(3))
        _weave(rest[n1:n2])
        _weave(rest[n2:-1], [f for p in range(NP) for f in mix_steps(p)],
               [lambda y: None] * 4 + [P(copy_x, t, j) for t in range(7) for j in range(8)])
        _weave(rest[-1:])

        @pl.when(jnp.logical_and(rep == 1, seg > 0))
        def _():
            out_copy(prev).start()

    def reset():
        mt_s[...] = jnp.zeros(mt_s.shape, F32)
        z_s[...] = jnp.zeros(z_s.shape, F32)

    x_copy(0).start()
    x_copy(1).start()

    gate = jax.nn.sigmoid(beta_ref[...].astype(F32).reshape(1, H))
    diag = lax.broadcasted_iota(jnp.int32, (H, H), 0) == lax.broadcasted_iota(jnp.int32, (H, H), 1)
    gate = jnp.sum(jnp.where(diag, jnp.broadcast_to(gate, (H, H)), 0.0), axis=1, keepdims=True)
    gate_s[...] = jnp.broadcast_to(gate, (H, 128))
    reset()
    for j in range(2):
        w_copy(j, 0).start()
        x_copy(j).wait()
        widen(0, j * L // 2, L // 2)
        for f in ln_steps(0, j * C, C, xs.at[0], j * C // 2, 0):
            f(None)
    w_copy(2, 0).start()
    w_copy(0, 0).wait()
    for f in prep_v_steps(0, 0):
        f(None)
    if cfg('ONLY', 7) & 1:
        lax.fori_loop(0, NP, P(a_body, True), None)
    for j in range(4, 2 * NSEG):
        x_copy(j).wait()
    lax.fori_loop(0, 2 * NC, lambda j, _: widen(2 + j // NC, j % NC * C, C), None)
    for t in range(3):
        b_copy(t).wait()
    for p in range(NP):
        w_copy(4, p).wait()

    def layer_pair(rep, _):
        if cfg('ONLY', 7) & 2:
            lax.fori_loop(NP - NP * rep, NSEG * NP, P(a_body, False), None)
        reset()
        k_b[:, L:] = jnp.zeros((NG, HALO, 128), F32)
        v_b[:, L:] = jnp.zeros((NG, HALO, 128), F32)
        if cfg('ONLY', 7) & 4:
            lax.fori_loop(0, NSEG, P(b_body, rep), None)
    lax.fori_loop(0, 2, layer_pair, None)

    def last(p, _):
        _weave(out_steps(NSEG - 1, 1, os_.at[1], p, True))
        last_copy(p).start()
    lax.fori_loop(0, NP, last, None)
    for s in range(NSEG - 1):
        out_copy(s).wait()
    for p in range(NP):
        last_copy(p).wait()


@jax.jit
def pallas_interleave_layers__memory_aug_infini_attn__sliding_local_dilated__prompt_kernel(
        A_x, A_wq, A_wk, A_wv, A_wo, A_beta, B_x, B_wqkv, B_wo):
    del B_x
    hbm = pl.BlockSpec(memory_space=pl.ANY)
    V = pltpu.VMEM
    T7 = 7 * 128
    scratch = [
        V((S, D), BF16),
        *[V((NP + 1, D, 256), BF16)] * 5,
        V((4, D, D), BF16),
        V((2, H * (DH + 2), 128), U32),
        V((NP, KH // 2, T7), U32), V((NP, KH // 2, T7), U32),
        V((NP, NP, 64, T7), U32), V((3 * NP, NP, 64, T7), U32),
        V((2, NP, KH // 2, T7), U32),
        V((H, 128), F32), V((NSEG + 1, L, D), F32),
        V((8, L // 4, KH), U32), V((2, 7, L // 4, KH), U32),
        V((2, NP, L // 4, T7), U32), V((NP, L // 4, T7), U32),
        V((NG, 128, 128), F32), V((NG, 8, 128), F32),
        V((2, L // 2, 256), U32), V((2, L // 2, 256), U32), V((2, 64, L), U32),
        [V((3, L, 128), F32)] * NP, V((NG, L + HALO, 128), F32), V((NG, L + HALO, 128), F32),
        V((W + 1, L, 128), F32), V((W + 1, L, 128), F32),
        [V((5, c * C + 64, 128), F32) for c in range(NC) for _ in range(2)],
        pltpu.SemaphoreType.DMA((2 * NSEG,)), pltpu.SemaphoreType.DMA((NSEG - 1 + NP,)),
        pltpu.SemaphoreType.DMA((5 * NP + 3,)),
    ]
    return pl.pallas_call(
        _kernel,
        in_specs=[hbm, pl.BlockSpec(memory_space=pltpu.VMEM), hbm, hbm, hbm, hbm, hbm, hbm],
        out_specs=hbm,
        out_shape=jax.ShapeDtypeStruct(A_x.shape, A_x.dtype),
        scratch_shapes=scratch,
        compiler_params=pltpu.CompilerParams(
            vmem_limit_bytes=110 * 2 ** 20,
            flags={os.environ['KCFG_FLAG']: True} if 'KCFG_FLAG' in os.environ else None),
        name="interleaved_attn",
    )(A_x, A_beta, A_wq, A_wk, A_wv, A_wo, B_wqkv, B_wo)
```

```python
import functools
import math

import jax
import jax.numpy as jnp
import numpy as np
from jax import lax
from jax.experimental import pallas as pl
from jax.experimental.pallas import tpu as pltpu

S, D, H, DH = 2048, 1024, 32, 32
L = 512
NSEG = S // L
NG = D // 128
NP = NG // 2
C = 128
NC = L // C
KH = D // 2
W, DIL = 8, 2
HALO = 16
LOG2E = math.log2(math.e)
QSCALE = DH ** -0.5 * LOG2E
MASKED = -1e9 * LOG2E
F32, BF16, U32 = jnp.float32, jnp.bfloat16, jnp.uint32
NN = (((1,), (0,)), ((), ()))
NT = (((1,), (1,)), ((), ()))
P = functools.partial

PLAN_FIRST = ("E01 Q03 q3 Q01x q4xx E10 Q12xx Q10 q5x q6xx R0x E11 Q13x Q11 E00x Q02xx Q00x R1xx U0xx U1xx", 128, 32, 2)
PLAN = ("E01 Q03 q3 Q01x q4x E10 Q12xx Q10 q5x q6x Q02xx R0x E00 Q00 Q13xxx R1 o0x E11 o1x o2x U0 Q11x o3 o4xxx o5 U1x o6", 216, 48, 4)


def _mm(a, b, dims=NN):
    return lax.dot_general(a, b, dims, preferred_element_type=F32)


def _pack(*xs):
    return pltpu.bitcast(jnp.concatenate(xs, axis=1).astype(BF16), U32)


def _bf(x):
    return pltpu.bitcast(x, BF16)


def _bits(x):
    return lax.bitcast_convert_type(x.astype(F32), U32)


def _join(lo, hi):
    return (_bits(lo) >> 16) | _bits(hi)


def _split(p):
    return (lax.bitcast_convert_type(p << 16, F32),
            lax.bitcast_convert_type(p & np.uint32(0xFFFF0000), F32))


def _iota(shape, axis):
    return lax.broadcasted_iota(jnp.int32, shape, axis)


def _layernorm(x):
    m = jnp.mean(x, axis=-1, keepdims=True)
    xc = x - m
    v = jnp.mean(xc * xc, axis=-1, keepdims=True)
    return xc * lax.rsqrt(v + 1e-5)


def _phi(t):
    return jnp.where(t > 0, t + 1.0, jnp.exp(t))


def _cross(xs):
    block = _iota(xs[0].shape, 1) // 32
    for bit in (1, 2):
        xs = [jnp.where(block & bit == 0, xs[i], xs[i ^ bit]) for i in range(4)]
    return xs


def _cross_rows(y):
    return jnp.concatenate(_cross([y[i * 32:(i + 1) * 32] for i in range(4)]), axis=0)


def _x_terms(x11, x12, x21, x22):
    return (x11 + x22, x21 + x22, x11, x22, x11 + x12, x21 - x11, x12 - x22)


def _w_terms(w11, w12, w21, w22):
    return (w11 + w22, w11, w12 - w22, w21 - w11, w22, w11 + w12, w21 + w22)


def _strassen_steps(prod, emit):
    m = {}

    def step(i):
        y = prod(i)
        if i == 1:
            m[1] = y
        elif i == 3:
            m[3] = y
            emit(1, 0, m[1] + y)
        elif i == 4:
            m[4] = y
            m["a"] = m.pop(3) - y
        elif i == 2:
            emit(0, 1, y + m.pop(4))
            m["b"] = y - m.pop(1)
        elif i == 0:
            m["a"] += y
            m["b"] += y
        elif i == 6:
            emit(0, 0, m.pop("a") + y)
        else:
            emit(1, 1, m.pop("b") + y)
        return y
    return [P(step, i) for i in (1, 3, 4, 2, 0, 6, 5)]


def _weave(mxu, *side):
    after = [[] for _ in mxu]
    for steps in side:
        for i, f in enumerate(steps):
            pos = (i + 0.5) / len(steps) * len(mxu)
            after[int(pos)].append((pos % 1.0, f))
    for f, todo in zip(mxu, after):
        y = f()
        for frac, g in sorted(todo, key=lambda t: t[0]):
            r = int(frac * (y.shape[0] // 8)) * 8
            g(y[r:r + 8, :128])


def _idle(n):
    return [lambda y: None] * n


def _pace(ref, y):
    if y is not None:
        if ref.dtype == BF16:
            y = jnp.concatenate([y, y], axis=0)
        ref[:y.shape[0], :128] = _bits(y) if ref.dtype == U32 else y.astype(ref.dtype)


def _ds(start, size, align=None):
    if not isinstance(start, int):
        start = pl.multiple_of(start, align or size)
    return pl.ds(start, size)


def _tile(g, n=1):
    return _ds(g * 128, n * 128, 128)


def _rows(c):
    return pl.ds(c * C, C)


def _packed_rows(c):
    return pl.ds(c * C // 2, C // 2)


def _k_tiles(ref, n):
    return _bf(jnp.concatenate([ref[kt, :, _tile(n)] for kt in range(NP)], axis=1))


def _kernel(x_h, beta_ref, awq_h, awk_h, awv_h, awo_h, bwqkv_h, bwo_h, out_h,
            io_s, raw_q, raw_k, raw_v, raw_ao, raw_bo, raw_b, tmp_s, wa_q, wa_k, wa_v, wb, wo,
            gate_s, x_s, x_new, xs, os_, o_cur, o_new, mt_s, z_s, q_a, k_a, vt_a,
            q_b, k_b, v_b, lg_b, p_b, sc, e_s, acc_s, sem_x, sem_o, sem_w):
    def x_copy(j):
        r = _ds(j * (L // 2), L // 2)
        return pltpu.make_async_copy(x_h.at[0, r], io_s.at[r], sem_x.at[j])

    def out_copy(s):
        r = _ds(s * L, L)
        return pltpu.make_async_copy(io_s.at[r], out_h.at[0, r], sem_o.at[s])

    def last_copy(p):
        r, c = pl.ds(S - L, L), _tile(2 * p, 2)
        return pltpu.make_async_copy(io_s.at[r, c], out_h.at[0, r, c], sem_o.at[NSEG - 1 + p])

    WV, WK, WQ, WAO, WBO = range(5)

    def w_copy(i, p):
        src, dst = ((awv_h, raw_v), (awk_h, raw_k), (awq_h, raw_q), (awo_h, raw_ao), (bwo_h, raw_bo))[i]
        return pltpu.make_async_copy(src.at[:, _tile(2 * p, 2)], dst.at[p], sem_w.at[i * NP + p])

    def b_copy(t):
        return pltpu.make_async_copy(bwqkv_h.at[:, _ds(t * D, D)], raw_b.at[t], sem_w.at[5 * NP + t])

    def ln_steps(s, r0, n, dst, d0, zero):
        def f(i, y):
            _pace(x_s.at[NSEG + zero], y)
            r = r0 + i * 16
            a = (r // C) * (2 * C) + r % C
            y1 = _layernorm(x_s[s, _ds(a, 16)])
            y2 = _layernorm(x_s[s, _ds(a + C, 16)])
            for t, v in enumerate(_x_terms(y1[:, :KH], y1[:, KH:], y2[:, :KH], y2[:, KH:])):
                dst.at[t][_ds(d0 + i * 8, 8)] = _pack(v)
        return [P(f, i) for i in range(n // 16)]

    def widen(s, dst, a, n):
        x_s[dst, _ds(a, n)] = io_s[_ds(s * L + a, n)].astype(F32)

    def pair_terms(w1, w2):
        w1, w2 = w1.astype(F32), w2.astype(F32)
        return _pack(*_w_terms(w1[:, :128], w1[:, 128:], w2[:, :128], w2[:, 128:]))

    def prep_qk_steps(raw, dst, p, zero):
        def f(k0, y):
            _pace(raw.at[NP + zero], y)
            dst.at[p][pl.ds(k0 // 2, 16)] = pair_terms(raw[p, pl.ds(k0, 32)], raw[p, pl.ds(KH + k0, 32)])
        return [P(f, k0) for k0 in range(0, KH, 32)]

    def prep_ao_steps(p, zero):
        def f(kp, k0, y):
            _pace(raw_ao.at[NP + zero], y)
            wo.at[0, p][pl.ds(kp * 64 + k0 // 2, 16)] = pair_terms(
                raw_ao[p, pl.ds(kp * 256 + k0, 32)], raw_ao[p, pl.ds(kp * 256 + 128 + k0, 32)])
        return [P(f, kp, k0) for kp in range(NP) for k0 in range(0, 128, 32)]

    def prep_v_steps(p, zero):
        def f(kt, n, y):
            _pace(raw_v.at[NP + zero], y)
            tmp_s[0, _tile(2 * kt + n)] = _join(raw_v[p, _tile(kt), _tile(n)], raw_v[p, _tile(NP + kt), _tile(n)]).T

        def h(kt, r, y):
            _pace(tmp_s.at[1 + zero], y)
            (w11, w21), (w12, w22) = (_split(tmp_s[0, pl.ds((2 * kt + n) * 128 + r, 32)]) for n in range(2))
            wa_v.at[p, kt][pl.ds(r // 2, 16)] = _pack(*_w_terms(w11, w12, w21, w22))
        return ([P(f, kt, n) for kt in range(NP) for n in range(2)]
                + [P(h, kt, r) for kt in range(NP) for r in range(0, 128, 32)])

    def spread(g, v):
        for h in range(4):
            tmp_s[0, pl.ds((4 * g + h) * (DH + 1), DH)] = v[h * DH:(h + 1) * DH]

    def gather(g, d):
        return tmp_s[0, pl.ds(4 * g + d, H, stride=DH + 1)]

    def prep_bo_steps(p, zero):
        def f(g, y):
            _pace(raw_bo.at[NP + zero], y)
            w = raw_bo[p, _tile(g)]
            spread(g, _join(w[:, :128], w[:, 128:]))

        def h(kp, d, y):
            _pace(tmp_s.at[1 + zero], y)
            (w11, w12), (w21, w22) = _split(gather(2 * kp, d)), _split(gather(2 * kp + 1, d))
            wo.at[1, p][pl.ds(kp * 64 + d * 16, 16)] = _pack(*_w_terms(w11, w12, w21, w22))
        return [P(f, g) for g in range(NG)] + [P(h, kp, d) for kp in range(NP) for d in range(4)]

    def prep_b_steps(t, kt, zero):
        def f(g, y):
            _pace(raw_b.at[3 + zero], y)
            spread(g, _join(raw_b[t, _tile(kt), _tile(g)], raw_b[t, _tile(NP + kt), _tile(g)]).T)

        def h(p, d, y):
            _pace(tmp_s.at[1 + zero], y)
            (w11, w21), (w12, w22) = _split(gather(2 * p, d)), _split(gather(2 * p + 1, d))
            wb.at[t * NP + p, kt][pl.ds(d * 16, 16)] = _pack(*_w_terms(w11, w12, w21, w22))
        return [P(f, g) for g in range(NG)] + [P(h, p, d) for p in range(NP) for d in range(4)]

    def out_steps(s, layer, o_terms, p, narrow=False):
        def emit(rh, nh, y):
            for i in range(2):
                c = 2 * i + rh
                x = x_s[s, _rows(c), _tile(2 * p + nh)] + y[i * C:(i + 1) * C]
                x_s[s, _rows(c), _tile(2 * p + nh)] = x
                if narrow:
                    io_s[_ds(s * L + c * C, C), _tile(2 * p + nh)] = x.astype(io_s.dtype)
        return _strassen_steps(lambda n: _mm(_k_tiles(o_terms, n), _bf(wo[layer, p, :, _tile(n)])), emit)

    same_head = _iota((128, 128), 1) // DH == _iota((128, 128), 0) // DH
    causal = _iota((32, 128), 0) <= _iota((32, 128), 1) % 32
    head64, block64 = _iota((64, 128), 1) // DH, _iota((64, 128), 0) // 16
    head_row = _iota((16, 128), 1) // DH == _iota((16, 128), 0)

    def a_body(first, rep, i, carry):
        seg, p = (0, i) if first else (i // NP, i % NP)
        slot = seg % 2
        zero = i // (NSEG * NP)
        live = {}

        def accumulate(key, v, op=jnp.add):
            live[key] = op(live[key], v) if key in live else v

        def qk_steps(is_k):
            def emit(rh, t, y):
                if not is_k:
                    y = jnp.concatenate([_cross_rows(y[:C]), _cross_rows(y[C:])], axis=0)
                ph = _phi(y)
                if is_k:
                    accumulate(("z", t), jnp.sum(ph.reshape(-1, 8, 128), axis=0))
                dst, y = (k_a, y) if is_k else (q_a, y * QSCALE)
                for j in range(2):
                    dst.at[t][_packed_rows(2 * j + rh)] = _pack(y[j * C:(j + 1) * C], ph[j * C:(j + 1) * C])
            w = wa_k if is_k else wa_q
            return _strassen_steps(lambda n: _mm(_bf(xs[slot, n]), _bf(w[p, :, _tile(n)])), emit)

        def v_steps():
            def emit(rh, t, y):
                vt_a.at[t][:, _tile(2 * rh, 2)] = _pack(y)
            return _strassen_steps(lambda n: _mm(_k_tiles(wa_v.at[p], n), _bf(xs[slot, n]), NT), emit)

        def vt(t, r, c):
            return vt_a[t, r, _tile(c % 2 * 2 + c // 2)]

        def queries(t, c, j):
            qc = q_a[t, _packed_rows(c), :128]
            return jnp.where(head64 == j ^ block64, qc, jnp.zeros_like(qc))

        def keep(t, c, j, r0, st):
            n = st.shape[0]
            if r0 + n == c * C + 32 * j + 32:
                sd = jnp.where(causal, st[n - 32:], -jnp.inf)
                st = sd if n == 32 else jnp.concatenate([st[:n - 32], sd], axis=0)
            accumulate(("max", t, c, j), jnp.max(st.reshape(-1, 8, 128), axis=0), jnp.maximum)
            accumulate(("keys", t, c, j), n, int.__add__)
            sc[2 * c + t][j, r0:r0 + n] = st

        def scores(t, c):
            st = _mm(_bf(k_a[t, :c * 64 + 16, :128]),
                     _bf(jnp.concatenate([queries(t, c, j) for j in range(4)], axis=0)), NT)
            for j in range(4):
                keep(t, c, j, 0, st[:, j * 128:(j + 1) * 128])
            return st

        def edge_scores(t, rh):
            ys = []
            for j in (3, 2, 1):
                for c in (rh, rh + 2):
                    ys.append(_mm(_bf(k_a[t, pl.ds(c * 64 + 16, 16 * j), :128]), _bf(queries(t, c, j)), NT))
                    keep(t, c, j, c * C + 32, ys[-1])
            return ys[0]

        def mem_read(t):
            g = 2 * p + t
            z = jnp.broadcast_to(jnp.sum(z_s[g], axis=0, keepdims=True), (16, 128))
            mz = jnp.concatenate([mt_s[g], jnp.where(head_row, z, 0.0)], axis=0).astype(BF16)
            live["mem", t] = _mm(mz, _bf(q_a[t, :, 128:]), NT)
            return live["mem", t]

        def mem_update(t):
            assert ("mem", t) in live
            g = 2 * p + t
            y = _mm(_bf(jnp.concatenate([vt(t, slice(None), c) for c in range(NC)], axis=1)), _bf(k_a[t, :, 128:]))
            mt_s[g] += jnp.where(same_head, y, 0.0)
            z_s[g] += live.pop(("z", t))
            return y

        def mix(t, c, kt, ys):
            if kt == 0:
                for j in range(4):
                    assert live["keys", t, c, j] == c * C + 32 * j + 32
                    live["max", t, c, j] = jnp.max(live["max", t, c, j], axis=0, keepdims=True)
            parts = {}
            for b in (3, 2, 1, 0):
                _pace(sc[2 * c + t].at[4 + zero], ys[3 - b])
                e = []
                for j in range(4):
                    if kt == c and b > j:
                        e.append(jnp.zeros((32, 128), F32))
                        continue
                    e.append(jnp.exp2(sc[2 * c + t][j, pl.ds(kt * C + b * 32, 32)] - live["max", t, c, j]))
                    accumulate(("sum", t, c, j), jnp.sum(e[-1].reshape(-1, 8, 128), axis=0))
                e_s[...] = _pack(*e)
                parts[b] = _cross([e_s[:, _tile(j)] for j in range(4)])
            for h in range(4):
                o = _mm(_bf(vt(t, pl.ds(h * DH // 2, DH // 2), kt)),
                        _bf(jnp.concatenate([parts[b][h] for b in range(4)], axis=0)))
                acc_s[2 * c + t, h] = acc_s[2 * c + t, h] + o if kt else o
            if kt == c:
                live["norm", t, c] = _cross([jnp.sum(live.pop(("sum", t, c, j)), axis=0, keepdims=True)
                                             for j in range(4)])

        def finish():
            for t in range(2):
                for c in range(NC):
                    if ("mem", t) in live and ("norm", t, c) in live:
                        mem = live["mem", t][:, c * C:(c + 1) * C]
                        outs = []
                        for h, norm in enumerate(live.pop(("norm", t, c))):
                            gate = gate_s[pl.ds((2 * p + t) * 4 + h, 1), :]
                            den = mem[128 + h:128 + h + 1] + 1e-6
                            outs.append(acc_s[2 * c + t, h] * ((1.0 - gate) / norm)
                                        + mem[h * DH:(h + 1) * DH] * (gate / den))
                        live["o", t, c] = _cross_rows(jnp.concatenate(outs, axis=0).T)
            for j in range(2):
                quad = [("o", t, 2 * j + rh) for rh in range(2) for t in range(2)]
                if all(n in live for n in quad):
                    o_new.at[0][_packed_rows(j)] = _pack(*_x_terms(*[live.pop(n) for n in quad]))

        def file_o(j, y):
            _pace(o_new.at[1 + zero], y)
            r = pl.ds(j * 16, 16)
            os_[(i + 2 * NP - 1) // NP % 2, (i + NP - 1) % NP, r] = o_new[0, r]

        def file_x(t, y):
            _pace(x_new.at[7 + zero], y)
            xs[1 - slot, t, _ds(p * 32, 32)] = x_new[t, :32]

        def widen_step(j, y):
            _pace(io_s.at[_ds(zero * 16, 16)], y)
            dst = 1 if first else jnp.where(rep == 0, seg + 1, NSEG)
            widen((seg + 1) % NSEG, dst, p // 2 * 256 + p % 2 * 64 + j % 2 * C + j // 2 * 16, 16)

        plan, lag, gap, slack = PLAN_FIRST if first else PLAN
        ln = ln_steps((seg + 1) % NSEG, p * 64, 64, x_new, 0, zero)
        ln = [f for j in range(4) for f in (P(widen_step, 2 * j), P(widen_step, 2 * j + 1), ln[j])] + _idle(slack)
        filing = [P(file_o, j) for j in range(8)]
        v, q, k = v_steps(), qk_steps(False), qk_steps(True)
        if first:
            out = None
            order = ((0, 3), (0, 1), (1, 2), (1, 0), (1, 3), (1, 1), (0, 2), (0, 0))
            nxt = jnp.minimum(p + 1, NP - 1)

            @pl.when(p == 0)
            def _():
                w_copy(WV, 1).start()
                x_copy(2).start()
                w_copy(WAO, 0).start()
            w_copy(WK, p).wait()
            w_copy(WQ, p).wait()
            _weave(v[:6], prep_qk_steps(raw_k, wa_k, p, zero) + prep_qk_steps(raw_q, wa_q, p, zero))
            _weave(v[6:])
            pl.when(p < NP - 1)(lambda: w_copy(WV, nxt).wait())
            pl.when(p % 2 == 0)(lambda: x_copy(2 + p // 2).wait())

            @pl.when(p < NP - 1)
            def _():
                for n in (WK, WQ, WAO):
                    w_copy(n, nxt).start()
            pl.when(p < NP - 2)(lambda: w_copy(WV, jnp.minimum(p + 2, NP - 1)).start())
            w_copy(WBO, p).start()
            pl.when(p == 0)(lambda: x_copy(3).start())
            x_copy(4 + p).start()
            pl.when(p > 0)(lambda: b_copy(jnp.maximum(p - 1, 0)).start())
            w_copy(WAO, p).wait()
            _weave(k + q[:3], prep_v_steps(nxt, zero), prep_ao_steps(p, zero) + _idle(2), ln, filing)
        else:
            out = out_steps((seg + NSEG - 1) % NSEG, jnp.where(seg == 0, 1, 0), os_.at[1 - slot], p)
            order = ((0, 3), (0, 1), (1, 2), (1, 0), (0, 2), (0, 0), (1, 3), (1, 1))
            prep = prep_b_steps(jnp.maximum(seg - 1, 0), p, zero) + prep_bo_steps(p, zero)
            _weave(k + v + q[:3], ln, prep, filing)

        jobs = [(t, c, kt) for t, c in order for kt in range(c + 1)]
        seen = []

        def plan_step(word):
            name = word.rstrip("x")
            args = [int(ch) for ch in name[1:]]
            if name[0] in "qo":
                y = (q if name[0] == "q" else out)[args[0]]()
            else:
                y = {"E": edge_scores, "Q": scores, "R": mem_read, "U": mem_update}[name[0]](*args)
            seen.extend((y, r) for r in range(0, y.shape[0], 8))
            for left in range(len(word) - len(name), 0, -1):
                marks = [seen[max(0, len(seen) - (lag + gap * (4 * left - b)) // 8)] for b in range(4)]
                mix(*jobs.pop(0), [m[r:r + 8, :128] for m, r in marks])
            finish()
            return y
        _weave([P(plan_step, word) for word in plan.split()], _idle(7) + [P(file_x, t) for t in range(7)])
        assert not jobs

    def b_body(rep, seg, carry):
        zero = seg // NSEG

        def proj_steps(t, p):
            def emit(rh, nh, y):
                for i in range(2):
                    c = 2 * i + rh
                    yi = y[i * C:(i + 1) * C]
                    if t == 0:
                        q_b[p][nh, _rows(c)] = yi * QSCALE
                        continue
                    dst, g = (k_b, v_b)[t - 1], 2 * p + nh
                    if c == NC - 1:
                        dst[g, :HALO] = dst[g, L:]
                    dst[g, pl.ds(HALO + c * C, C)] = yi
            return _strassen_steps(lambda n: _mm(_bf(xs[0, n]), _k_tiles(wb.at[t * NP + p], n), NT), emit)

        def shifted(ref, g, r0, w):
            return ref[g, pl.ds(r0 + HALO - DIL * w, 8)]

        def logit_steps(p):
            def f(r0, y):
                _pace(q_b[p].at[2 + zero], y)
                lg = []
                for w in range(W):
                    acc = None if p == 0 else lg_b[w, r0:r0 + 8]
                    for n in range(2):
                        t = q_b[p][n, r0:r0 + 8] * shifted(k_b, 2 * p + n, r0, w)
                        acc = t if acc is None else acc + t
                    if p < NP - 1:
                        lg_b[w, r0:r0 + 8] = acc
                        continue
                    acc = acc + pltpu.roll(acc, 64, 1)
                    acc = acc + pltpu.roll(acc, 32, 1)
                    if r0 < DIL * w:
                        acc = jnp.where(seg * L + r0 + _iota((8, 128), 0) >= DIL * w, acc, MASKED)
                    lg.append(acc)
                if lg:
                    m = functools.reduce(jnp.maximum, lg)
                    e = [jnp.exp2(t - m) for t in lg]
                    inv = 1.0 / functools.reduce(jnp.add, e)
                    for w in range(W):
                        p_b[w, r0:r0 + 8] = e[w] * inv
            return [P(f, r0) for r0 in range(0, L, 8)]

        def o_home(p):
            return os_.at[1, p] if p < NP - 1 else o_new.at[0]

        def mix_steps(p):
            part = []

            def f(r, j, y):
                _pace(p_b.at[W + zero], y)
                r0 = r // C * 2 * C + r % C + j // 2 * C + j % 2 * 8
                pw = [p_b[w, r0:r0 + 8] for w in range(W)]
                part.append([functools.reduce(jnp.add, [pw[w] * shifted(v_b, g, r0, w) for w in range(W)])
                             for g in (2 * p, 2 * p + 1)])
                if j == 3:
                    quad = [jnp.concatenate([part[2 * a][b], part[2 * a + 1][b]], axis=0)
                            for a in range(2) for b in range(2)]
                    part.clear()
                    o_home(p)[pl.ds(r // 2, 8)] = _pack(*_x_terms(*quad))
            return [P(f, r, j) for r in range(0, L // 2, 16) for j in range(4)]

        def take_o(p, j, y):
            _pace(os_.at[zero, 0] if p < NP - 1 else o_new.at[1 + zero], y)
            o_cur[p, pl.ds(j * 16, 16)] = o_home(p)[pl.ds(j * 16, 16)]

        def file_x(t, j, y):
            _pace(x_new.at[7 + zero], y)
            xs[0, t, pl.ds(j * 16, 16)] = x_new[t, pl.ds(j * 16, 16)]

        prev = (seg + NSEG - 1) % NSEG
        out = [f for p in range(NP) for f in out_steps(prev, jnp.where(seg == 0, 0, 1), o_cur, p, True)]
        take = [P(take_o, p, j) for p in range(NP) for j in range(8)]
        _weave(proj_steps(2, 0) + proj_steps(0, 0) + proj_steps(1, 0),
               ln_steps((seg + 1) % NSEG, 0, L // 2, x_new, 0, zero))
        _weave(proj_steps(0, 1) + proj_steps(1, 1), logit_steps(0), take[:12])
        _weave(proj_steps(0, 2) + proj_steps(1, 2), logit_steps(1), take[12:22])
        _weave(proj_steps(0, 3) + proj_steps(1, 3), logit_steps(2), take[22:])
        values = proj_steps(2, 1) + proj_steps(2, 2) + proj_steps(2, 3)
        mixes = [f for p in range(NP) for f in mix_steps(p)]
        _weave(values[:17], logit_steps(3))
        _weave(values[17:19])
        _weave(values[19:], mixes[:18])
        _weave(out[:-1], mixes[18:], [P(file_x, t, j) for t in range(7) for j in range(8)])
        _weave(out[-1:])

        @pl.when(jnp.logical_and(rep == 1, seg > 0))
        def _():
            out_copy(prev).start()

    def clear_memory():
        mt_s[...] = jnp.zeros(mt_s.shape, F32)
        z_s[...] = jnp.zeros(z_s.shape, F32)

    x_copy(0).start()
    x_copy(1).start()
    gate = jnp.broadcast_to(jax.nn.sigmoid(beta_ref[...].astype(F32).reshape(1, H)), (H, H))
    gate = jnp.sum(jnp.where(_iota((H, H), 0) == _iota((H, H), 1), gate, 0.0), axis=1, keepdims=True)
    gate_s[...] = jnp.broadcast_to(gate, (H, 128))
    clear_memory()
    o_new[0] = jnp.zeros(o_new.shape[1:], U32)
    for j in range(2):
        w_copy((WV, WK)[j], 0).start()
        x_copy(j).wait()
        widen(0, 0, j * L // 2, L // 2)
        for f in ln_steps(0, j * C, C, xs.at[0], j * C // 2, 0):
            f(None)
    w_copy(WQ, 0).start()
    w_copy(WV, 0).wait()
    for f in prep_v_steps(0, 0):
        f(None)
    lax.fori_loop(0, NP, P(a_body, True, 0), None)
    for j in range(4, 2 * NSEG):
        x_copy(j).wait()
    for t in range(3):
        b_copy(t).wait()
    for p in range(NP):
        w_copy(WBO, p).wait()

    def layer_pair(rep, carry):
        lax.fori_loop(NP - NP * rep, NSEG * NP, P(a_body, False, rep), None)
        clear_memory()
        k_b[:, L:] = jnp.zeros((NG, HALO, 128), F32)
        v_b[:, L:] = jnp.zeros((NG, HALO, 128), F32)
        lax.fori_loop(0, NSEG, P(b_body, rep), None)
    lax.fori_loop(0, 2, layer_pair, None)

    os_[1, NP - 1] = o_new[0]

    def last(p, carry):
        _weave(out_steps(NSEG - 1, 1, os_.at[1], p, True))
        last_copy(p).start()
    lax.fori_loop(0, NP, last, None)
    for s in range(NSEG - 1):
        out_copy(s).wait()
    for p in range(NP):
        last_copy(p).wait()


@jax.jit
def pallas_interleave_layers__memory_aug_infini_attn__sliding_local_dilated__prompt_kernel(
    A_x: jax.Array,
    A_wq: jax.Array,
    A_wk: jax.Array,
    A_wv: jax.Array,
    A_wo: jax.Array,
    A_beta: jax.Array,
    B_x: jax.Array,
    B_wqkv: jax.Array,
    B_wo: jax.Array,
):
    del B_x
    hbm = pl.BlockSpec(memory_space=pl.ANY)
    V = pltpu.VMEM
    T7 = 7 * 128
    scratch = [
        V((S, D), BF16),
        *[V((NP + 1, D, 256), BF16)] * 5,
        V((4, D, D), BF16),
        V((2, H * (DH + 2), 128), U32),
        V((NP, KH // 2, T7), U32), V((NP, KH // 2, T7), U32),
        V((NP, NP, 64, T7), U32), V((3 * NP, NP, 64, T7), U32),
        V((2, NP, KH // 2, T7), U32),
        V((H, 128), F32), V((NSEG + 1, L, D), F32),
        V((8, L // 4, KH), U32), V((2, 7, L // 4, KH), U32),
        V((2, NP, L // 4, T7), U32), V((NP, L // 4, T7), U32),
        V((2, L // 4, T7), U32),
        V((NG, 128, 128), F32), V((NG, 8, 128), F32),
        V((2, L // 2, 256), U32), V((2, L // 2, 256), U32),
        V((2, 64, L), U32),
        [V((3, L, 128), F32)] * NP,
        V((NG, L + HALO, 128), F32), V((NG, L + HALO, 128), F32),
        V((W, L, 128), F32), V((W + 1, L, 128), F32),
        [V((5, c * C + C, 128), F32) for c in range(NC) for _ in range(2)],
        V((16, 512), U32), V((2 * NC, 4, DH, 128), F32),
        pltpu.SemaphoreType.DMA((2 * NSEG,)),
        pltpu.SemaphoreType.DMA((NSEG - 1 + NP,)),
        pltpu.SemaphoreType.DMA((5 * NP + 3,)),
    ]
    return pl.pallas_call(
        _kernel,
        in_specs=[hbm, pl.BlockSpec(memory_space=pltpu.VMEM), hbm, hbm, hbm, hbm, hbm, hbm],
        out_specs=hbm,
        out_shape=jax.ShapeDtypeStruct(A_x.shape, A_x.dtype),
        scratch_shapes=scratch,
        compiler_params=pltpu.CompilerParams(vmem_limit_bytes=110 * 2 ** 20),
        name="interleaved_attn",
    )(A_x, A_beta, A_wq, A_wk, A_wv, A_wo, B_wqkv, B_wo)
```

```python
import functools
import math

import jax
import jax.numpy as jnp
import numpy as np
from jax import lax
from jax.experimental import pallas as pl
from jax.experimental.pallas import tpu as pltpu

S, D, H, DH = 2048, 1024, 32, 32
L = 512
NSEG = S // L
NG = D // 128
NP = NG // 2
C = 128
NC = L // C
KH = D // 2
W, DIL = 8, 2
HALO = 16
LOG2E = math.log2(math.e)
QSCALE = DH ** -0.5 * LOG2E
MASKED = -1e9 * LOG2E
F32, BF16, U32 = jnp.float32, jnp.bfloat16, jnp.uint32
NN = (((1,), (0,)), ((), ()))
NT = (((1,), (1,)), ((), ()))
P = functools.partial

PLAN_FIRST = ("Q03 E01 q3x Q01x q4 Q10 E10xx Q12x q5x q6xx R0x Q13 E11x E00 Q11 R1xx Q02xxx U0xx Q00x U1xx", 168, 32, 2)
PLAN = ("E01 Q03 q3 Q01x q4x E10 Q12xx q5x q6x Q10 Q02xx R0x E00 Q00x Q13xx R1 o0x o1x E11 U0 o2x Q11x o3 o4xxx o5x U1 o6", 248, 60, 1)


def _mm(a, b, dims=NN):
    return lax.dot_general(a, b, dims, preferred_element_type=F32)


def _pack(*xs):
    return pltpu.bitcast(jnp.concatenate(xs, axis=1).astype(BF16), U32)


def _bf(x):
    return pltpu.bitcast(x, BF16)


def _bits(x):
    return lax.bitcast_convert_type(x.astype(F32), U32)


def _join(lo, hi):
    return (_bits(lo) >> 16) | _bits(hi)


def _split(p):
    return (lax.bitcast_convert_type(p << 16, F32),
            lax.bitcast_convert_type(p & np.uint32(0xFFFF0000), F32))


def _iota(shape, axis):
    return lax.broadcasted_iota(jnp.int32, shape, axis)


def _layernorm(x):
    m = jnp.mean(x, axis=-1, keepdims=True)
    xc = x - m
    v = jnp.mean(xc * xc, axis=-1, keepdims=True)
    return xc * lax.rsqrt(v + 1e-5)


def _phi(t):
    return jnp.where(t > 0, t + 1.0, jnp.exp(t))


def _x_terms(x11, x12, x21, x22):
    return (x11 + x22, x21 + x22, x11, x22, x11 + x12, x21 - x11, x12 - x22)


def _w_terms(w11, w12, w21, w22):
    return (w11 + w22, w11, w12 - w22, w21 - w11, w22, w11 + w12, w21 + w22)


def _strassen_steps(prod, emit):
    m = {}

    def step(i):
        y = prod(i)
        if i == 1:
            m[1] = y
        elif i == 3:
            m[3] = y
            emit(1, 0, m[1] + y)
        elif i == 4:
            m[4] = y
            m["a"] = m.pop(3) - y
        elif i == 2:
            emit(0, 1, y + m.pop(4))
            m["b"] = y - m.pop(1)
        elif i == 0:
            m["a"] += y
            m["b"] += y
        elif i == 6:
            emit(0, 0, m.pop("a") + y)
        else:
            emit(1, 1, m.pop("b") + y)
        return y
    return [P(step, i) for i in (1, 3, 4, 2, 0, 6, 5)]


def _weave(mxu, *side):
    after = [[] for _ in mxu]
    for steps in side:
        for i, f in enumerate(steps):
            pos = (i + 0.5) / len(steps) * len(mxu)
            after[int(pos)].append((pos % 1.0, f))
    for f, todo in zip(mxu, after):
        y = f()
        for frac, g in sorted(todo, key=lambda t: t[0]):
            r = int(frac * (y.shape[0] // 8)) * 8
            g(y[r:r + 8, :128])


def _idle(n):
    return [lambda y: None] * n


def _pace(ref, y):
    if y is not None:
        if ref.dtype == BF16:
            y = jnp.concatenate([y, y], axis=0)
        ref[:y.shape[0], :128] = _bits(y) if ref.dtype == U32 else y.astype(ref.dtype)


def _ds(start, size, align=None):
    if not isinstance(start, int):
        start = pl.multiple_of(start, align or size)
    return pl.ds(start, size)


def _tile(g, n=1):
    return _ds(g * 128, n * 128, 128)


def _rows(c):
    return pl.ds(c * C, C)


def _packed_rows(c):
    return pl.ds(c * C // 2, C // 2)


def _k_tiles(ref, n):
    return _bf(jnp.concatenate([ref[kt, :, _tile(n)] for kt in range(NP)], axis=1))


def _kernel(x_h, beta_ref, awq_h, awk_h, awv_h, awo_h, bwqkv_h, bwo_h, out_h,
            io_s, raw_q, raw_k, raw_v, raw_ao, raw_bo, raw_b, tmp_s, wa_q, wa_k, wa_v, wb, wo,
            gate_s, x_s, x_new, xs, os_, o_cur, o_new, mt_s, z_s, q_a, k_a, vt_a,
            q_b, k_b, v_b, lg_b, p_b, sc, e_s, acc_s, sem_x, sem_o, sem_w):
    def x_copy(j):
        r = _ds(j * (L // 2), L // 2)
        return pltpu.make_async_copy(x_h.at[0, r], io_s.at[r], sem_x.at[j])

    def out_copy(s):
        r = _ds(s * L, L)
        return pltpu.make_async_copy(io_s.at[r], out_h.at[0, r], sem_o.at[s])

    def last_copy(p):
        r, c = pl.ds(S - L, L), _tile(2 * p, 2)
        return pltpu.make_async_copy(io_s.at[r, c], out_h.at[0, r, c], sem_o.at[NSEG - 1 + p])

    WV, WK, WQ, WAO, WBO = range(5)

    def w_copy(i, p):
        src, dst = ((awv_h, raw_v), (awk_h, raw_k), (awq_h, raw_q), (awo_h, raw_ao), (bwo_h, raw_bo))[i]
        return pltpu.make_async_copy(src.at[:, _tile(2 * p, 2)], dst.at[p], sem_w.at[i * NP + p])

    def b_copy(t):
        return pltpu.make_async_copy(bwqkv_h.at[:, _ds(t * D, D)], raw_b.at[t], sem_w.at[5 * NP + t])

    def ln_steps(s, r0, n, dst, d0, zero):
        def f(i, y):
            _pace(x_s.at[NSEG + zero], y)
            r = r0 + i * 16
            a = (r // C) * (2 * C) + r % C
            y1 = _layernorm(x_s[s, _ds(a, 16)])
            y2 = _layernorm(x_s[s, _ds(a + C, 16)])
            for t, v in enumerate(_x_terms(y1[:, :KH], y1[:, KH:], y2[:, :KH], y2[:, KH:])):
                dst.at[t][_ds(d0 + i * 8, 8)] = _pack(v)
        return [P(f, i) for i in range(n // 16)]

    def widen(s, dst, a, n):
        x_s[dst, _ds(a, n)] = io_s[_ds(s * L + a, n)].astype(F32)

    def pair_terms(w1, w2):
        w1, w2 = w1.astype(F32), w2.astype(F32)
        return _pack(*_w_terms(w1[:, :128], w1[:, 128:], w2[:, :128], w2[:, 128:]))

    def prep_qk_steps(raw, dst, p, zero):
        def f(k0, y):
            _pace(raw.at[NP + zero], y)
            dst.at[p][pl.ds(k0 // 2, 16)] = pair_terms(raw[p, pl.ds(k0, 32)], raw[p, pl.ds(KH + k0, 32)])
        return [P(f, k0) for k0 in range(0, KH, 32)]

    def prep_ao_steps(p, zero):
        def f(kp, k0, y):
            _pace(raw_ao.at[NP + zero], y)
            wo.at[0, p][pl.ds(kp * 64 + k0 // 2, 16)] = pair_terms(
                raw_ao[p, pl.ds(kp * 256 + k0, 32)], raw_ao[p, pl.ds(kp * 256 + 128 + k0, 32)])
        return [P(f, kp, k0) for kp in range(NP) for k0 in range(0, 128, 32)]

    def prep_v_steps(p, zero):
        def f(kt, n, y):
            _pace(raw_v.at[NP + zero], y)
            tmp_s[0, _tile(2 * kt + n)] = _join(raw_v[p, _tile(kt), _tile(n)], raw_v[p, _tile(NP + kt), _tile(n)]).T

        def h(kt, r, y):
            _pace(tmp_s.at[1 + zero], y)
            (w11, w21), (w12, w22) = (_split(tmp_s[0, pl.ds((2 * kt + n) * 128 + r, 32)]) for n in range(2))
            wa_v.at[p, kt][pl.ds(r // 2, 16)] = _pack(*_w_terms(w11, w12, w21, w22))
        return ([P(f, kt, n) for kt in range(NP) for n in range(2)]
                + [P(h, kt, r) for kt in range(NP) for r in range(0, 128, 32)])

    def spread(g, v):
        for h in range(4):
            tmp_s[0, pl.ds((4 * g + h) * (DH + 1), DH)] = v[h * DH:(h + 1) * DH]

    def gather(g, d):
        return tmp_s[0, pl.ds(4 * g + d, H, stride=DH + 1)]

    def prep_bo_steps(p, zero):
        def f(g, y):
            _pace(raw_bo.at[NP + zero], y)
            w = raw_bo[p, _tile(g)]
            spread(g, _join(w[:, :128], w[:, 128:]))

        def h(kp, d, y):
            _pace(tmp_s.at[1 + zero], y)
            (w11, w12), (w21, w22) = _split(gather(2 * kp, d)), _split(gather(2 * kp + 1, d))
            wo.at[1, p][pl.ds(kp * 64 + d * 16, 16)] = _pack(*_w_terms(w11, w12, w21, w22))
        return [P(f, g) for g in range(NG)] + [P(h, kp, d) for kp in range(NP) for d in range(4)]

    def prep_b_steps(t, kt, zero):
        def f(g, y):
            _pace(raw_b.at[3 + zero], y)
            spread(g, _join(raw_b[t, _tile(kt), _tile(g)], raw_b[t, _tile(NP + kt), _tile(g)]).T)

        def h(p, d, y):
            _pace(tmp_s.at[1 + zero], y)
            (w11, w21), (w12, w22) = _split(gather(2 * p, d)), _split(gather(2 * p + 1, d))
            wb.at[t * NP + p, kt][pl.ds(d * 16, 16)] = _pack(*_w_terms(w11, w12, w21, w22))
        return [P(f, g) for g in range(NG)] + [P(h, p, d) for p in range(NP) for d in range(4)]

    def out_steps(s, layer, o_terms, p, narrow=False):
        def emit(rh, nh, y):
            for i in range(2):
                c = 2 * i + rh
                x = x_s[s, _rows(c), _tile(2 * p + nh)] + y[i * C:(i + 1) * C]
                x_s[s, _rows(c), _tile(2 * p + nh)] = x
                if narrow:
                    io_s[_ds(s * L + c * C, C), _tile(2 * p + nh)] = x.astype(io_s.dtype)
        return _strassen_steps(lambda n: _mm(_k_tiles(o_terms, n), _bf(wo[layer, p, :, _tile(n)])), emit)

    same_head = _iota((128, 128), 1) // DH == _iota((128, 128), 0) // DH
    causal = _iota((32, 128), 0) <= _iota((32, 128), 1) % 32
    head64, block64 = _iota((64, 128), 1) // DH, _iota((64, 128), 0) // 16
    head_row = _iota((16, 128), 1) // DH == _iota((16, 128), 0)
    stay = {(n, bit): _iota((n, 128), 1) & (32 * bit) == 0 for n in (1, 16, 32) for bit in (1, 2)}

    def cross(vs):
        for bit in (1, 2):
            vs = [lax.select(stay[vs[0].shape[0], bit], vs[i], vs[i ^ bit]) for i in range(4)]
        return vs

    def cross_rows(y):
        return jnp.concatenate(cross([y[i * 32:(i + 1) * 32] for i in range(4)]), axis=0)

    def a_body(first, rep, i, carry):
        seg, p = (0, i) if first else (i // NP, i % NP)
        slot = seg % 2
        zero = i // (NSEG * NP)
        live = {}

        def accumulate(key, v, op=jnp.add):
            live[key] = op(live[key], v) if key in live else v

        def qk_steps(is_k):
            def emit(rh, t, y):
                if not is_k:
                    y = jnp.concatenate([cross_rows(y[:C]), cross_rows(y[C:])], axis=0)
                ph = _phi(y)
                if is_k:
                    accumulate(("z", t), jnp.sum(ph.reshape(-1, 8, 128), axis=0))
                dst, y = (k_a, y) if is_k else (q_a, y * QSCALE)
                for j in range(2):
                    dst.at[t][_packed_rows(2 * j + rh)] = _pack(y[j * C:(j + 1) * C], ph[j * C:(j + 1) * C])
            w = wa_k if is_k else wa_q
            return _strassen_steps(lambda n: _mm(_bf(xs[slot, n]), _bf(w[p, :, _tile(n)])), emit)

        def v_steps():
            def emit(rh, t, y):
                vt_a.at[t][:, _tile(2 * rh, 2)] = _pack(y)
            return _strassen_steps(lambda n: _mm(_k_tiles(wa_v.at[p], n), _bf(xs[slot, n]), NT), emit)

        def vt(t, r, c):
            return vt_a[t, r, _tile(c % 2 * 2 + c // 2)]

        def queries(t, c, j):
            qc = q_a[t, _packed_rows(c), :128]
            return jnp.where(head64 == j ^ block64, qc, jnp.zeros_like(qc))

        def keep(t, c, j, r0, st):
            n = st.shape[0]
            if r0 + n == c * C + 32 * j + 32:
                sd = jnp.where(causal, st[n - 32:], -jnp.inf)
                st = sd if n == 32 else jnp.concatenate([st[:n - 32], sd], axis=0)
            accumulate(("max", t, c, j), jnp.max(st.reshape(-1, 8, 128), axis=0), jnp.maximum)
            accumulate(("keys", t, c, j), n, int.__add__)
            sc[2 * c + t][j, r0:r0 + n] = st

        def scores(t, c):
            st = _mm(_bf(k_a[t, :c * 64 + 16, :128]),
                     _bf(jnp.concatenate([queries(t, c, j) for j in range(4)], axis=0)), NT)
            for j in range(4):
                keep(t, c, j, 0, st[:, j * 128:(j + 1) * 128])
            return st

        def edge_scores(t, rh):
            ys = []
            for j in (3, 2, 1):
                for c in (rh, rh + 2):
                    ys.append(_mm(_bf(k_a[t, pl.ds(c * 64 + 16, 16 * j), :128]), _bf(queries(t, c, j)), NT))
                    keep(t, c, j, c * C + 32, ys[-1])
            return ys[0]

        def mem_read(t):
            g = 2 * p + t
            z = jnp.broadcast_to(jnp.sum(z_s[g], axis=0, keepdims=True), (16, 128))
            mz = jnp.concatenate([mt_s[g], jnp.where(head_row, z, 0.0)], axis=0).astype(BF16)
            live["mem", t] = _mm(mz, _bf(q_a[t, :, 128:]), NT)
            return live["mem", t]

        def mem_update(t):
            assert ("mem", t) in live
            g = 2 * p + t
            y = _mm(_bf(jnp.concatenate([vt(t, slice(None), c) for c in range(NC)], axis=1)), _bf(k_a[t, :, 128:]))
            mt_s[g] += jnp.where(same_head, y, 0.0)
            z_s[g] += live.pop(("z", t))
            return y

        def mix(t, c, kt, ys):
            if kt == 0:
                for j in range(4):
                    assert live["keys", t, c, j] == c * C + 32 * j + 32
                    live["max", t, c, j] = jnp.max(live["max", t, c, j], axis=0, keepdims=True)
            parts = {}
            for b in (3, 2, 1, 0):
                _pace(sc[2 * c + t].at[4 + zero], ys[3 - b])
                e = []
                for j in range(4):
                    if kt == c and b > j:
                        e.append(jnp.zeros((32, 128), F32))
                        continue
                    e.append(jnp.exp2(sc[2 * c + t][j, pl.ds(kt * C + b * 32, 32)] - live["max", t, c, j]))
                    accumulate(("sum", t, c, j), jnp.sum(e[-1].reshape(-1, 8, 128), axis=0))
                e_s[...] = _pack(*e)
                parts[b] = cross([e_s[:, _tile(j)] for j in range(4)])
            for h in range(4):
                o = _mm(_bf(vt(t, pl.ds(h * DH // 2, DH // 2), kt)),
                        _bf(jnp.concatenate([parts[b][h] for b in range(4)], axis=0)))
                acc_s[2 * c + t, h] = acc_s[2 * c + t, h] + o if kt else o
            if kt == c:
                live["norm", t, c] = cross([jnp.sum(live.pop(("sum", t, c, j)), axis=0, keepdims=True)
                                             for j in range(4)])

        def finish():
            for t in range(2):
                for c in range(NC):
                    if ("mem", t) in live and ("norm", t, c) in live:
                        mem = live["mem", t][:, c * C:(c + 1) * C]
                        outs = []
                        for h, norm in enumerate(live.pop(("norm", t, c))):
                            gate = gate_s[pl.ds((2 * p + t) * 4 + h, 1), :]
                            den = mem[128 + h:128 + h + 1] + 1e-6
                            outs.append(acc_s[2 * c + t, h] * ((1.0 - gate) / norm)
                                        + mem[h * DH:(h + 1) * DH] * (gate / den))
                        live["o", t, c] = cross_rows(jnp.concatenate(outs, axis=0).T)
            for j in range(2):
                quad = [("o", t, 2 * j + rh) for rh in range(2) for t in range(2)]
                if all(n in live for n in quad):
                    o_new.at[0][_packed_rows(j)] = _pack(*_x_terms(*[live.pop(n) for n in quad]))

        def file_o(j, y):
            _pace(o_new.at[1 + zero], y)
            r = pl.ds(j * 16, 16)
            os_[(i + 2 * NP - 1) // NP % 2, (i + NP - 1) % NP, r] = o_new[0, r]

        def file_x(t, y):
            _pace(x_new.at[7 + zero], y)
            xs[1 - slot, t, _ds(p * 32, 32)] = x_new[t, :32]

        def widen_step(j, y):
            _pace(io_s.at[_ds(zero * 16, 16)], y)
            dst = 1 if first else jnp.where(rep == 0, seg + 1, NSEG)
            widen((seg + 1) % NSEG, dst, p // 2 * 256 + p % 2 * 64 + j % 2 * C + j // 2 * 16, 16)

        plan, lag, gap, slack = PLAN_FIRST if first else PLAN
        ln = ln_steps((seg + 1) % NSEG, p * 64, 64, x_new, 0, zero)
        ln = [f for j in range(4) for f in (P(widen_step, 2 * j), P(widen_step, 2 * j + 1), ln[j])] + _idle(slack)
        filing = [P(file_o, j) for j in range(8)]
        v, q, k = v_steps(), qk_steps(False), qk_steps(True)
        if first:
            out = None
            order = ((0, 3), (0, 1), (1, 2), (1, 0), (1, 3), (1, 1), (0, 2), (0, 0))
            nxt = jnp.minimum(p + 1, NP - 1)

            @pl.when(p == 0)
            def _():
                w_copy(WV, 1).start()
                x_copy(2).start()
                w_copy(WAO, 0).start()
            w_copy(WK, p).wait()
            w_copy(WQ, p).wait()
            _weave(v[:6], prep_qk_steps(raw_k, wa_k, p, zero) + prep_qk_steps(raw_q, wa_q, p, zero))
            _weave(v[6:])
            pl.when(p < NP - 1)(lambda: w_copy(WV, nxt).wait())
            pl.when(p % 2 == 0)(lambda: x_copy(2 + p // 2).wait())

            @pl.when(p < NP - 1)
            def _():
                for n in (WK, WQ, WAO):
                    w_copy(n, nxt).start()
            pl.when(p < NP - 2)(lambda: w_copy(WV, jnp.minimum(p + 2, NP - 1)).start())
            w_copy(WBO, p).start()
            pl.when(p == 0)(lambda: x_copy(3).start())
            x_copy(4 + p).start()
            pl.when(p > 0)(lambda: b_copy(jnp.maximum(p - 1, 0)).start())
            w_copy(WAO, p).wait()
            _weave(k + q[:3], prep_v_steps(nxt, zero), prep_ao_steps(p, zero) + _idle(2), ln, filing)
        else:
            out = out_steps((seg + NSEG - 1) % NSEG, jnp.where(seg == 0, 1, 0), os_.at[1 - slot], p)
            order = ((0, 3), (0, 1), (1, 2), (1, 0), (0, 2), (0, 0), (1, 3), (1, 1))
            prep = prep_b_steps(jnp.maximum(seg - 1, 0), p, zero) + prep_bo_steps(p, zero)
            _weave(k + v + q[:3], ln, prep, filing)

        jobs = [(t, c, kt) for t, c in order for kt in range(c + 1)]
        seen = []

        def plan_step(word):
            name = word.rstrip("x")
            args = [int(ch) for ch in name[1:]]
            if name[0] in "qo":
                y = (q if name[0] == "q" else out)[args[0]]()
            else:
                y = {"E": edge_scores, "Q": scores, "R": mem_read, "U": mem_update}[name[0]](*args)
            seen.extend((y, r) for r in range(0, y.shape[0], 8))
            for left in range(len(word) - len(name), 0, -1):
                marks = [seen[max(0, len(seen) - (lag + gap * (4 * left - b)) // 8)] for b in range(4)]
                mix(*jobs.pop(0), [m[r:r + 8, :128] for m, r in marks])
            finish()
            return y
        _weave([P(plan_step, word) for word in plan.split()], _idle(7) + [P(file_x, t) for t in range(7)])
        assert not jobs

    def b_body(rep, seg, carry):
        zero = seg // NSEG

        def proj_steps(t, p):
            def emit(rh, nh, y):
                for i in range(2):
                    c = 2 * i + rh
                    yi = y[i * C:(i + 1) * C]
                    if t == 0:
                        q_b[p][nh, _rows(c)] = yi * QSCALE
                        continue
                    dst, g = (k_b, v_b)[t - 1], 2 * p + nh
                    if c == NC - 1:
                        dst[g, :HALO] = dst[g, L:]
                    dst[g, pl.ds(HALO + c * C, C)] = yi
            return _strassen_steps(lambda n: _mm(_bf(xs[0, n]), _k_tiles(wb.at[t * NP + p], n), NT), emit)

        def window(ref, p, r0):
            taps = [ref[2 * p:2 * p + 2, pl.ds(r0 + HALO - DIL * w, 8)] for w in range(W)]
            return jnp.concatenate(taps, axis=0).reshape(W, 2, 8, 128)

        def logit_steps(p):
            def f(r0, y):
                _pace(q_b[p].at[2 + zero], y)
                lg = jnp.sum(window(k_b, p, r0) * q_b[p][:2, r0:r0 + 8], axis=1)
                if p > 0:
                    lg = lg + lg_b[:, r0:r0 + 8]
                if p < NP - 1:
                    lg_b[:, r0:r0 + 8] = lg
                    return
                lg = lg + pltpu.roll(lg, 64, 2)
                lg = lg + pltpu.roll(lg, 32, 2)
                if r0 < HALO:
                    lg = jnp.where(seg * L + r0 + _iota(lg.shape, 1) >= DIL * _iota(lg.shape, 0), lg, MASKED)
                e = jnp.exp2(lg - jnp.max(lg, axis=0))
                p_b[:W, r0:r0 + 8] = e * (1.0 / jnp.sum(e, axis=0))
            return [P(f, r0) for r0 in range(0, L, 8)]

        def o_home(p):
            return os_.at[1, p] if p < NP - 1 else o_new.at[0]

        def mix_steps(p):
            part = []

            def f(r, j, y):
                _pace(p_b.at[W + zero], y)
                r0 = r // C * 2 * C + r % C + j // 2 * C + j % 2 * 8
                part.append(jnp.sum(window(v_b, p, r0) * p_b[:W, r0:r0 + 8][:, None], axis=0))
                if j == 3:
                    o1, o2 = jnp.concatenate(part[:2], axis=1), jnp.concatenate(part[2:], axis=1)
                    part.clear()
                    o_home(p)[pl.ds(r // 2, 8)] = _pack(*_x_terms(o1[0], o1[1], o2[0], o2[1]))
            return [P(f, r, j) for r in range(0, L // 2, 16) for j in range(4)]

        def take_o(p, j, y):
            _pace(os_.at[zero, 0] if p < NP - 1 else o_new.at[1 + zero], y)
            o_cur[p, pl.ds(j * 16, 16)] = o_home(p)[pl.ds(j * 16, 16)]

        def file_x(t, j, y):
            _pace(x_new.at[7 + zero], y)
            xs[0, t, pl.ds(j * 16, 16)] = x_new[t, pl.ds(j * 16, 16)]

        prev = (seg + NSEG - 1) % NSEG
        out = [f for p in range(NP) for f in out_steps(prev, jnp.where(seg == 0, 0, 1), o_cur, p, True)]
        take = [P(take_o, p, j) for p in range(NP) for j in range(8)]
        _weave(proj_steps(2, 0) + proj_steps(0, 0) + proj_steps(1, 0),
               ln_steps((seg + 1) % NSEG, 0, L // 2, x_new, 0, zero))
        _weave(proj_steps(0, 1) + proj_steps(1, 1), logit_steps(0), take[:12])
        _weave(proj_steps(0, 2) + proj_steps(1, 2), logit_steps(1), take[12:22])
        _weave(proj_steps(0, 3) + proj_steps(1, 3), logit_steps(2), take[22:])
        values = proj_steps(2, 1) + proj_steps(2, 2) + proj_steps(2, 3)
        mixes = [f for p in range(NP) for f in mix_steps(p)]
        _weave(values[:17], logit_steps(3))
        _weave(values[17:19])
        _weave(values[19:], mixes[:18])
        _weave(out[:-1], mixes[18:], [P(file_x, t, j) for t in range(7) for j in range(8)])
        _weave(out[-1:])

        @pl.when(jnp.logical_and(rep == 1, seg > 0))
        def _():
            out_copy(prev).start()

    def clear_memory():
        mt_s[...] = jnp.zeros(mt_s.shape, F32)
        z_s[...] = jnp.zeros(z_s.shape, F32)

    x_copy(0).start()
    x_copy(1).start()
    gate = jnp.broadcast_to(jax.nn.sigmoid(beta_ref[...].astype(F32).reshape(1, H)), (H, H))
    gate = jnp.sum(jnp.where(_iota((H, H), 0) == _iota((H, H), 1), gate, 0.0), axis=1, keepdims=True)
    gate_s[...] = jnp.broadcast_to(gate, (H, 128))
    clear_memory()
    o_new[0] = jnp.zeros(o_new.shape[1:], U32)
    for j in range(2):
        w_copy((WV, WK)[j], 0).start()
        x_copy(j).wait()
        widen(0, 0, j * L // 2, L // 2)
        for f in ln_steps(0, j * C, C, xs.at[0], j * C // 2, 0):
            f(None)
    w_copy(WQ, 0).start()
    w_copy(WV, 0).wait()
    for f in prep_v_steps(0, 0):
        f(None)
    lax.fori_loop(0, NP, P(a_body, True, 0), None)
    for j in range(4, 2 * NSEG):
        x_copy(j).wait()
    for t in range(3):
        b_copy(t).wait()
    for p in range(NP):
        w_copy(WBO, p).wait()

    def layer_pair(rep, carry):
        lax.fori_loop(NP - NP * rep, NSEG * NP, P(a_body, False, rep), None)
        clear_memory()
        k_b[:, L:] = jnp.zeros((NG, HALO, 128), F32)
        v_b[:, L:] = jnp.zeros((NG, HALO, 128), F32)
        lax.fori_loop(0, NSEG, P(b_body, rep), None)
    lax.fori_loop(0, 2, layer_pair, None)

    os_[1, NP - 1] = o_new[0]

    def last(p, carry):
        _weave(out_steps(NSEG - 1, 1, os_.at[1], p, True))
        last_copy(p).start()
    lax.fori_loop(0, NP, last, None)
    for s in range(NSEG - 1):
        out_copy(s).wait()
    for p in range(NP):
        last_copy(p).wait()


@jax.jit
def pallas_interleave_layers__memory_aug_infini_attn__sliding_local_dilated__prompt_kernel(
    A_x: jax.Array,
    A_wq: jax.Array,
    A_wk: jax.Array,
    A_wv: jax.Array,
    A_wo: jax.Array,
    A_beta: jax.Array,
    B_x: jax.Array,
    B_wqkv: jax.Array,
    B_wo: jax.Array,
):
    del B_x
    hbm = pl.BlockSpec(memory_space=pl.ANY)
    V = pltpu.VMEM
    T7 = 7 * 128
    scratch = [
        V((S, D), BF16),
        *[V((NP + 1, D, 256), BF16)] * 5,
        V((4, D, D), BF16),
        V((2, H * (DH + 2), 128), U32),
        V((NP, KH // 2, T7), U32), V((NP, KH // 2, T7), U32),
        V((NP, NP, 64, T7), U32), V((3 * NP, NP, 64, T7), U32),
        V((2, NP, KH // 2, T7), U32),
        V((H, 128), F32), V((NSEG + 1, L, D), F32),
        V((8, L // 4, KH), U32), V((2, 7, L // 4, KH), U32),
        V((2, NP, L // 4, T7), U32), V((NP, L // 4, T7), U32),
        V((2, L // 4, T7), U32),
        V((NG, 128, 128), F32), V((NG, 8, 128), F32),
        V((2, L // 2, 256), U32), V((2, L // 2, 256), U32),
        V((2, 64, L), U32),
        [V((3, L, 128), F32)] * NP,
        V((NG, L + HALO, 128), F32), V((NG, L + HALO, 128), F32),
        V((W, L, 128), F32), V((W + 1, L, 128), F32),
        [V((5, c * C + C, 128), F32) for c in range(NC) for _ in range(2)],
        V((16, 512), U32), V((2 * NC, 4, DH, 128), F32),
        pltpu.SemaphoreType.DMA((2 * NSEG,)),
        pltpu.SemaphoreType.DMA((NSEG - 1 + NP,)),
        pltpu.SemaphoreType.DMA((5 * NP + 3,)),
    ]
    return pl.pallas_call(
        _kernel,
        in_specs=[hbm, pl.BlockSpec(memory_space=pltpu.VMEM), hbm, hbm, hbm, hbm, hbm, hbm],
        out_specs=hbm,
        out_shape=jax.ShapeDtypeStruct(A_x.shape, A_x.dtype),
        scratch_shapes=scratch,
        compiler_params=pltpu.CompilerParams(vmem_limit_bytes=110 * 2 ** 20),
        name="interleaved_attn",
    )(A_x, A_beta, A_wq, A_wk, A_wv, A_wo, B_wqkv, B_wo)
```
